```python
import jax
import jax.numpy as jnp

def _softmax(x, axis=-1):
    return jax.nn.softmax(x, axis=axis)
def _gelu(x):
    return jax.nn.gelu(x, approximate=True)
def _silu(x):
    return jax.nn.silu(x)
def _sigmoid(x):
    return jax.nn.sigmoid(x)
def _layernorm(x, axis=-1, eps=1e-5):
    m = jnp.mean(x, axis=axis, keepdims=True)
    v = jnp.var(x, axis=axis, keepdims=True)
    return (x - m) / jnp.sqrt(v + eps)
def _scatter_add(tgt, idx, src, axis=0):
    return tgt.at[idx].add(src)
def _segment_sum(src, seg, n):
    return jax.ops.segment_sum(src, seg, n)
class _Rng:
    def __init__(self, key):
        self._k = key
    def _next(self):
        self._k, sub = jax.random.split(self._k)
        return sub
    def normal(self, shape):
        return jax.random.normal(self._next(), shape, dtype=jnp.bfloat16)
    def randint(self, lo, hi, shape):
        return jax.random.randint(self._next(), shape, lo, hi, dtype=jnp.int32)
    def uniform(self, shape, lo=0.0, hi=1.0):
        return jax.random.uniform(self._next(), shape, jnp.bfloat16, lo, hi)
    def permutation(self, n):
        return jax.random.permutation(self._next(), n)


kernel_name = 'interleave_layers__sliding_local_dilated__softmax_full_mha__prompt'

def setup_inputs():
    _rng = _Rng(jax.random.key(int.from_bytes(__import__("os").urandom(4), "little")))
    _w = (lambda a: (lambda t: t.astype(jnp.bfloat16) if jnp.issubdtype(t.dtype, jnp.floating) else t)(jnp.asarray(a)))
    def _A_setup():
        B, S, D = 1, 2048, 1024
        return {
            "x": _w((lambda *s: _rng.normal(s) * 0.05)(B, S, D)),
            "wqkv": _w((lambda *s: _rng.normal(s) * 0.05)(D, 3 * D)),
            "wo": _w((lambda *s: _rng.normal(s) * 0.05)(D, D)),
        }
    _A_in = _A_setup()

    def _B_setup():
        B, S, D = 1, 2048, 1024
        return {
            "x": _w((lambda *s: _rng.normal(s) * 0.05)(B, S, D)),
            "wqkv": _w((lambda *s: _rng.normal(s) * 0.05)(D, 3 * D)),
            "wo": _w((lambda *s: _rng.normal(s) * 0.05)(D, D)),
        }
    _B_in = _B_setup()

    return {
        "A_x": _A_in["x"],
        "A_wqkv": _A_in["wqkv"],
        "A_wo": _A_in["wo"],
        "B_x": _B_in["x"],
        "B_wqkv": _B_in["wqkv"],
        "B_wo": _B_in["wo"],
    }

def reference(A_x, A_wqkv, A_wo, B_x, B_wqkv, B_wo):
    def _A_ref(x, wqkv, wo):
        B, S, D = x.shape
        H = 32; Dh = D // H
        W, dil = 8, 2
        qkv = (lambda x, *d: x.transpose(*d))((x @ wqkv).reshape(B, S, 3, H, Dh), 2, 0, 3, 1, 4)
        q, k, v = qkv[0], qkv[1], qkv[2]
        scale = Dh ** -0.5
        pos = jnp.arange(S)
        off = jnp.arange(W) * dil
        idx = pos[:, None] - off[None, :]
        mask = idx >= 0
        idx_c = jnp.where(mask, idx, 0).reshape(-1)
        kg = k[:, :, idx_c, :].reshape(B, H, S, W, Dh)
        vg = v[:, :, idx_c, :].reshape(B, H, S, W, Dh)
        logits = jnp.einsum("bhsd,bhswd->bhsw", q, kg) * scale
        logits = jnp.where(mask[None, None, :, :], logits, -1e9)
        attn = _softmax(logits, axis=-1)
        o = jnp.einsum("bhsw,bhswd->bhsd", attn, vg)
        return (lambda x, *d: x.transpose(*d))(o, 0, 2, 1, 3).reshape(B, S, D) @ wo

    def _B_ref(x, wqkv, wo):
        B, S, D = x.shape
        H = 32; Dh = D // H
        qkv = (lambda x, *d: x.transpose(*d))((x @ wqkv).reshape(B, S, 3, H, Dh), 2, 0, 3, 1, 4)
        q, k, v = qkv[0], qkv[1], qkv[2]
        scale = Dh ** -0.5
        scores = jnp.einsum("bhqd,bhkd->bhqk", q, k) * scale
        p = _softmax(scores, axis=-1)
        o = jnp.einsum("bhqk,bhkd->bhqd", p, v)
        return (lambda x, *d: x.transpose(*d))(o, 0, 2, 1, 3).reshape(B, S, D) @ wo

    x = A_x
    x = x + _A_ref(_layernorm(x, axis=-1), A_wqkv, A_wo)
    x = x + _B_ref(_layernorm(x, axis=-1), B_wqkv, B_wo)
    x = x + _A_ref(_layernorm(x, axis=-1), A_wqkv, A_wo)
    x = x + _B_ref(_layernorm(x, axis=-1), B_wqkv, B_wo)
    return x
```

```python
import math

import jax
import jax.numpy as jnp
from jax import lax
import jax.experimental.pallas as pl
import jax.experimental.pallas.tpu as pltpu

S = 2048
D = 1024
H = 32
DH = D // H
WIN = 8
NB = 8
BW = S // NB
NG = D // 128
EPS = 1e-5
LOG2E = math.log2(math.e)
QSCALE = DH ** -0.5 * LOG2E
NEG = -1e9 * LOG2E

AQ, AK, AV, AO, BQ, BK, BV, BO = (NG * i for i in range(8))

f32, bf16, u32 = jnp.float32, jnp.bfloat16, jnp.uint32


def _pack(x):
    return pltpu.bitcast(x.astype(bf16), u32)


def _unpack(x):
    return pltpu.bitcast(x, bf16)


def _interleave(*tasks):
    state = [[0, n, gen] for n, gen in tasks]
    while state:
        t = min(state, key=lambda t: (t[0] + 0.5) / t[1])
        try:
            next(t[2])
            t[0] += 1
        except StopIteration:
            state.remove(t)


def _kernel(x_hbm, awqkv, awo, bwqkv, bwo, o_hbm,
            xio, wraw, wt, xt, xn, qa, ka, va, qb, kb, vb, ob, sbuf, mbuf,
            xsem, wsem):
    w_hbm = (awqkv, awqkv, awqkv, awo, bwqkv, bwqkv, bwqkv, bwo)
    w_off = (0, NG, 2 * NG, 0, 0, NG, 2 * NG, 0)

    def cols(i):
        return pl.ds(pl.multiple_of(i * 128, 128), 128)

    def x_copy(f):
        return pltpu.make_async_copy(x_hbm.at[:, cols(f)], xio.at[f], xsem.at[f])

    def o_copy(f):
        return pltpu.make_async_copy(xio.at[f], o_hbm.at[:, cols(f)], xsem.at[f])

    def w_copy(m, g):
        return pltpu.make_async_copy(w_hbm[m].at[:, cols(w_off[m] + g)],
                                     wraw.at[m * NG + g], wsem.at[m * NG + g])

    def w_prep(n):
        wt[n] = pltpu.bitcast(wraw[n].T, u32)

    for f in range(NG):
        x_copy(f).start()
    for m in range(3):
        w_copy(m, 0).start()
    for g in range(NG):
        for m in range(8):
            if m >= 3:
                w_copy(m, g).start()
            elif g + 1 < NG:
                w_copy(m, g + 1).start()

    def zero_body(i, _):
        z = jnp.zeros((128, BW), f32)
        qa[1, jnp.minimum(i, NB - 1)] = z
        ka[1, i] = z
        va[1, i] = z
        return 0
    lax.fori_loop(0, 2 * NB - 1, zero_body, 0)

    xio_u = xio.bitcast(u32)

    def in_body(f, _):
        x_copy(f).wait()
        for c in range(NB):
            u = xio_u[f, pl.ds(c, 128, stride=NB), :].T
            xt[c, cols(f), 0:128] = pltpu.bitcast(u << 16, f32)
            xt[c, cols(f), 128:256] = pltpu.bitcast(u & jnp.uint32(0xFFFF0000), f32)
        return 0
    lax.fori_loop(0, NG, in_body, 0)
    for m in range(3):
        w_copy(m, 0).wait()
        w_prep(m * NG)

    def layernorm():
        def body(c, _):
            acc = xt[c, 0:32, :]
            for r in range(32, D, 32):
                acc = acc + xt[c, r:r + 32, :]
            mean = jnp.sum(acc, axis=0, keepdims=True) * (1.0 / D)
            acc = None
            for r in range(0, D, 32):
                d = xt[c, r:r + 32, :] - mean
                acc = d * d if acc is None else acc + d * d
            rstd = lax.rsqrt(jnp.sum(acc, axis=0, keepdims=True) * (1.0 / D) + EPS)
            for r in range(0, D, 32):
                xn[c, r // 2:r // 2 + 16, :] = _pack((xt[c, r:r + 32, :] - mean) * rstd)
            return 0
        lax.fori_loop(0, NB, body, 0)

    def proj(n, src, c):
        return jnp.dot(_unpack(wt[n]), _unpack(src[c]), preferred_element_type=f32)

    def qkv_a(g):
        slot = g % 2
        for c in range(NB):
            qa[slot, c] = proj(AQ + g, xn, c) * QSCALE
            yield
            for base, dst in ((AK, ka), (AV, va)):
                y = proj(base + g, xn, c)
                dst[slot, NB - 1 + c] = y
                if c > 0:
                    for par in range(2):
                        ls = slice(128 * par, 128 * par + 128)
                        dst[slot, c - 1, :, ls] = pltpu.roll(y[:, ls], 1, 1)
                yield

    def local_head(slot, rows, orows):
        first = lax.broadcasted_iota(jnp.int32, (1, 128), 1) == 0
        for c in range(NB):
            for par in range(2):
                ls = slice(128 * par, 128 * par + 128)
                q = qa[slot, c, rows, ls]
                t = []
                for w in range(WIN):
                    tw = jnp.sum(q * ka[slot, NB - 1 + c - w, rows, ls], axis=0, keepdims=True)
                    t.append(jnp.where(first, NEG, tw) if c < w else tw)
                m = t[0]
                for w in range(1, WIN):
                    m = jnp.maximum(m, t[w])
                l = o = None
                for w in range(WIN):
                    e = jnp.exp2(t[w] - m)
                    ev = e * va[slot, NB - 1 + c - w, rows, ls]
                    l = e if l is None else l + e
                    o = ev if o is None else o + ev
                ob[c, orows, ls] = _pack(o * (1.0 / l))
                yield

    def head_rows(h):
        return pl.ds(pl.multiple_of(h * (DH // 2), DH // 2), DH // 2)

    def local_group(g, slot):
        for hh in range(4):
            yield from local_head(slot, slice(hh * DH, (hh + 1) * DH), head_rows(4 * g + hh))

    def prep_task(g):
        nxt = jnp.minimum(g + 1, NG - 1)
        for m in range(7, -1, -1):
            w_prep(m * NG + (nxt if m < 3 else g))
            yield

    def layer_a(p):
        def body(g, _):
            @pl.when(p == 0)
            def _():
                for m in range(3, 8):
                    w_copy(m, g).wait()

                @pl.when(g + 1 < NG)
                def _():
                    for m in range(3):
                        w_copy(m, g + 1).wait()
            _interleave((3 * NB, qkv_a(g)),
                        (8 * NB, local_group(jnp.maximum(g - 1, 0), (g + 1) % 2)),
                        (8, prep_task(g)))
            return 0
        lax.fori_loop(0, NG, body, 0)

        def tail(hh, _):
            rows = pl.ds(pl.multiple_of(hh * DH, DH), DH)
            for _ in local_head((NG - 1) % 2, rows, head_rows(4 * (NG - 1) + hh)):
                pass
            return 0
        lax.fori_loop(0, 4, tail, 0)

        def out_body(f, _):
            for c in range(NB):
                xt[c, cols(f), :] += proj(AO + f, ob, c)
            return 0
        lax.fori_loop(0, NG, out_body, 0)

    KC = 128

    def full_step(h, hn):
        for qi in range(NB // 2):
            if hn is not None:
                q = jnp.concatenate([qb[2 * qi + i, head_rows(hn), :] for i in range(2)], axis=1)
                z = jnp.zeros_like(q)
                qp = _unpack(jnp.concatenate(
                    [jnp.where(hn % 4 == i, q, z) for i in range(4)], axis=0))
            if h is not None:
                mb = mbuf[qi]
            m = l = acc = None
            for j in range(S // KC):
                if h is not None:
                    pieces = [None] * (KC // 16)
                    for r in reversed(range(KC // 16)):
                        s = sbuf[qi, j * KC + r * 16:j * KC + r * 16 + 16, :]
                        e = jnp.exp2(s.reshape(2, 8, 2 * BW) - mb[None])
                        l = e[0] + e[1] if l is None else l + (e[0] + e[1])
                        pieces[r] = _pack(e.reshape(16, 2 * BW))
                    pt = _unpack(jnp.concatenate(pieces, axis=0))
                if hn is not None:
                    k = _unpack(kb[hn // 4, j * KC // 2:(j + 1) * KC // 2, :])
                    s = jnp.dot(k, qp, preferred_element_type=f32)
                    for r in range(KC // 8):
                        sr = s[r * 8:r * 8 + 8]
                        sbuf[qi, j * KC + r * 8:j * KC + r * 8 + 8, :] = sr
                        m = sr if m is None else jnp.maximum(m, sr)
                if h is not None:
                    v = _unpack(vb[j // 2, head_rows(h), (j % 2) * 128:(j % 2) * 128 + 128])
                    o = jnp.dot(v, pt, preferred_element_type=f32)
                    acc = o if acc is None else acc + o
            if h is not None:
                o = _pack(acc * (1.0 / jnp.sum(l, axis=0, keepdims=True)))
                for i in range(2):
                    ob[2 * qi + i, head_rows(h), :] = o[:, i * BW:(i + 1) * BW]
            if hn is not None:
                mbuf[qi] = jnp.broadcast_to(jnp.max(m, axis=0, keepdims=True), (8, 2 * BW))

    def layer_b(p):
        def body(g, _):
            rows = pl.ds(pl.multiple_of(g * 64, 64), 64)
            for c in range(NB):
                qb[c, rows, :] = _pack(proj(BQ + g, xn, c) * QSCALE)
                kt = proj(BK + g, xn, c).astype(bf16).T
                kb[g, c * BW // 2:(c + 1) * BW // 2, :] = pltpu.bitcast(kt, u32)
                vb[c, rows, :] = _pack(proj(BV + g, xn, c))
            return 0
        lax.fori_loop(0, NG, body, 0)

        full_step(None, 0)

        def head_body(h, _):
            full_step(h, h + 1)
            return 0
        lax.fori_loop(0, H - 1, head_body, 0)
        full_step(H - 1, None)

        def out_body(f, _):
            for c in range(NB):
                y = xt[c, cols(f), :] + proj(BO + f, ob, c)
                xt[c, cols(f), :] = y
                u = pltpu.pack_elementwise([y[:, :128], y[:, 128:]], packed_dtype=bf16)
                xio_u[f, pl.ds(c, 128, stride=NB), :] = pltpu.bitcast(u, u32).T

            @pl.when(p == 1)
            def _():
                o_copy(f).start()
            return 0
        lax.fori_loop(0, NG, out_body, 0)

    def period(p, _):
        layernorm()
        layer_a(p)
        layernorm()
        layer_b(p)
        return 0
    lax.fori_loop(0, 2, period, 0)

    for f in range(NG):
        o_copy(f).wait()


@jax.jit
def pallas_interleave_layers__sliding_local_dilated__softmax_full_mha__prompt_kernel(
    A_x: jax.Array,
    A_wqkv: jax.Array,
    A_wo: jax.Array,
    B_x: jax.Array,
    B_wqkv: jax.Array,
    B_wo: jax.Array,
):
    del B_x
    act = pltpu.VMEM((NB, D // 2, BW), u32)
    out = pl.pallas_call(
        _kernel,
        out_shape=jax.ShapeDtypeStruct((S, D), bf16),
        in_specs=[pl.BlockSpec(memory_space=pl.ANY)] * 5,
        out_specs=pl.BlockSpec(memory_space=pl.ANY),
        scratch_shapes=[
            pltpu.VMEM((NG, S, 128), bf16),
            pltpu.VMEM((8 * NG, D, 128), bf16),
            pltpu.VMEM((8 * NG, 64, D), u32),
            pltpu.VMEM((NB, D, BW), f32),
            act,
            pltpu.VMEM((2, NB, 128, BW), f32),
            pltpu.VMEM((2, 2 * NB - 1, 128, BW), f32),
            pltpu.VMEM((2, 2 * NB - 1, 128, BW), f32),
            act,
            pltpu.VMEM((NG, S // 2, 128), u32),
            act,
            act,
            pltpu.VMEM((NB // 2, S, 2 * BW), f32),
            pltpu.VMEM((NB // 2, 8, 2 * BW), f32),
            pltpu.SemaphoreType.DMA((NG,)),
            pltpu.SemaphoreType.DMA((8 * NG,)),
        ],
        compiler_params=pltpu.CompilerParams(vmem_limit_bytes=110 * 2**20),
        name="interleave_layers",
    )(A_x.reshape(S, D), A_wqkv, A_wo, B_wqkv, B_wo)
    return out.reshape(A_x.shape)
```

```python
import math

import jax
import jax.numpy as jnp
from jax import lax
import jax.experimental.pallas as pl
import jax.experimental.pallas.tpu as pltpu

S = 2048
D = 1024
H = 32
DH = D // H
WIN = 8
NB = 8
BW = S // NB
NG = D // 128
EPS = 1e-5
LOG2E = math.log2(math.e)
QSCALE = DH ** -0.5 * LOG2E
NEG = -1e9 * LOG2E

AQ, AK, AV, AO, BQ, BK, BV, BO = (NG * i for i in range(8))

f32, bf16, u32 = jnp.float32, jnp.bfloat16, jnp.uint32
HALF = (slice(0, 128), slice(128, 256))


def _pack2(lo, hi):
    return pltpu.bitcast(pltpu.pack_elementwise([lo, hi], packed_dtype=bf16), u32)


def _unpack2(u):
    return pltpu.bitcast(u << 16, f32), pltpu.bitcast(u & jnp.uint32(0xFFFF0000), f32)


def _zip16(x):
    m, n = x.shape
    x = x.reshape(m // 16, 2, 8, n)
    return _pack2(x[:, 0], x[:, 1]).reshape(m // 2, n)


def _bf(u):
    return pltpu.bitcast(u, bf16)


def _interleave(*tasks):
    state = [[0, n, gen] for n, gen in tasks]
    while state:
        t = min(state, key=lambda t: (t[0] + 0.5) / t[1])
        try:
            next(t[2])
            t[0] += 1
        except StopIteration:
            state.remove(t)


def _run(gen):
    for _ in gen:
        pass


def _ds(i, n):
    if isinstance(i, int):
        return pl.ds(i * n, n)
    return pl.ds(pl.multiple_of(i * n, n), n)


def _kernel(x_hbm, awqkv, awo, bwqkv, bwo, o_hbm,
            xio, wraw, wt, xt, xn, qa, ka, va, qb, kb, vb, ob, sbuf, mbuf,
            xsem, wsem):
    w_hbm = (awqkv, awqkv, awqkv, awo, bwqkv, bwqkv, bwqkv, bwo)
    w_off = (0, NG, 2 * NG, 0, 0, NG, 2 * NG, 0)

    def x_copy(f):
        return pltpu.make_async_copy(x_hbm.at[:, _ds(f, 128)], xio.at[f], xsem.at[f])

    def o_copy(f):
        return pltpu.make_async_copy(xio.at[f], o_hbm.at[:, _ds(f, 128)], xsem.at[f])

    def w_copy(m, g):
        return pltpu.make_async_copy(w_hbm[m].at[:, _ds(w_off[m] + g, 128)],
                                     wraw.at[m * NG + g], wsem.at[m * NG + g])

    def w_copies(g, action):
        for m in range(3, 8):
            action(w_copy(m, g))

        @pl.when(g + 1 < NG)
        def _():
            for m in range(3):
                action(w_copy(m, g + 1))

    def w_prep(n):
        for t in range(4):
            w = wraw[n, 256 * t:256 * t + 256, :].astype(f32).reshape(8, 4, 8, 128)
            k1, k2 = (pltpu.bitcast(
                _bf(_pack2(w[:, i], w[:, i + 1]).reshape(64, 128)).T, u32) for i in (0, 2))
            ls = slice(128 * t, 128 * t + 128)
            wt[n, 2, :, ls] = k1[:32]
            wt[n, 3, :, ls] = k2[32:]
            a11, a21, a12, a22 = (_unpack2(k) for k in (k1[:32], k1[32:], k2[:32], k2[32:]))
            for r, a, b, op in ((0, a11, a22, jnp.add), (1, a21, a22, jnp.add),
                                (4, a11, a12, jnp.add), (5, a21, a11, jnp.subtract),
                                (6, a12, a22, jnp.subtract)):
                wt[n, r, :, ls] = _pack2(op(a[0], b[0]), op(a[1], b[1]))
            yield

    def put_act(dst, c, h, even, odd):
        b11, b21, b12, b22 = even[:16], even[16:], odd[:16], odd[16:]
        for r, t in enumerate((b11 + b22, b11, b12 - b22, b21 - b11, b22, b11 + b12, b21 + b22)):
            dst[c, r, _ds(h, 8), :] = _pack2(t[:8], t[8:])

    def proj(n, src, c, emit):
        def mm(r):
            return jnp.dot(_bf(wt[n, r]), _bf(src[c, r]), preferred_element_type=f32)
        m2 = mm(1)
        yield
        m4 = mm(3)
        emit(1, 0, m2 + m4)
        yield
        t22 = mm(5) - m2
        yield
        t11 = mm(6) + m4
        yield
        m1 = mm(0)
        t11, t22 = t11 + m1, t22 + m1
        yield
        m3 = mm(2)
        emit(1, 1, t22 + m3)
        yield
        m5 = mm(4)
        emit(0, 1, m3 + m5)
        emit(0, 0, t11 - m5)
        yield

    for f in range(NG):
        x_copy(f).start()
    for m in range(3):
        w_copy(m, 0).start()

    def zero_body(i, _):
        z = jnp.zeros((128, BW), f32)
        qa[1, jnp.minimum(i, NB - 1)] = z
        ka[1, i] = z
        va[1, i] = z
        return 0
    lax.fori_loop(0, 2 * NB - 1, zero_body, 0)

    xio_u = xio.bitcast(u32)

    def in_body(f, _):
        x_copy(f).wait()
        for c in range(NB):
            even, odd = _unpack2(xio_u[f, pl.ds(c, 128, stride=NB), :].T)
            xt[c, _ds(f, 128), HALF[0]] = even
            xt[c, _ds(f, 128), HALF[1]] = odd
        return 0
    lax.fori_loop(0, NG, in_body, 0)
    w_copies(0, lambda cp: cp.start())
    for m in range(3):
        w_copy(m, 0).wait()
    _interleave(*((4, w_prep(m * NG)) for m in range(3)))

    def layernorm(c):
        acc = None
        for h in range(H):
            x = xt[c, _ds(h, DH), :]
            acc = x if acc is None else acc + x
            if h % 8 == 7:
                yield
        mean = jnp.sum(acc, axis=0, keepdims=True) * (1.0 / D)
        acc = None
        for h in range(H):
            d = xt[c, _ds(h, DH), :] - mean
            acc = d * d if acc is None else acc + d * d
            if h % 8 in (2, 5, 7):
                yield
        rstd = lax.rsqrt(jnp.sum(acc, axis=0, keepdims=True) * (1.0 / D) + EPS)
        for h in range(H):
            y = (xt[c, _ds(h, DH), :] - mean) * rstd
            put_act(xn, c, h, y[:, HALF[0]], y[:, HALF[1]])
            yield

    def layernorm_from(first):
        def ln_body(c, _):
            _run(layernorm(c))
            return 0
        lax.fori_loop(first, NB, ln_body, 0)

    def residual(n, c, f):
        def emit(i, par, y):
            xt[c, _ds(2 * f + i, 64), HALF[par]] += y
        return proj(n, ob, c, emit)

    def out_proj(base):
        def block(c):
            for f in range(NG):
                yield from residual(base + f, c, f)

        def out_body(c, _):
            _interleave((7 * NG, block(c)), (48, layernorm(jnp.maximum(c - 1, 0))))
            return 0
        lax.fori_loop(0, NB, out_body, 0)

    def qkv_a(g):
        slot = g % 2
        for c in range(NB):
            def emit_q(i, par, y):
                qa[slot, c, _ds(i, 64), HALF[par]] = y * QSCALE
            yield from proj(AQ + g, xn, c, emit_q)
            for base, dst in ((AK, ka), (AV, va)):
                def emit_kv(i, par, y):
                    dst[slot, NB - 1 + c, _ds(i, 64), HALF[par]] = y
                    if c > 0:
                        dst[slot, c - 1, _ds(i, 64), HALF[par]] = pltpu.roll(y, 1, 1)
                yield from proj(base + g, xn, c, emit_kv)

    def local_head(slot, hh, h):
        first = lax.broadcasted_iota(jnp.int32, (1, 128), 1) == 0
        rows = _ds(hh, DH)
        for c in range(NB):
            out = []
            for ls in HALF:
                q = qa[slot, c, rows, ls]
                t = []
                for w in range(WIN):
                    tw = jnp.sum(q * ka[slot, NB - 1 + c - w, rows, ls], axis=0, keepdims=True)
                    t.append(jnp.where(first, NEG, tw) if c < w else tw)
                m = t[0]
                for w in range(1, WIN):
                    m = jnp.maximum(m, t[w])
                yield
                l = o = None
                for w in range(WIN):
                    e = jnp.exp2(t[w] - m)
                    ev = e * va[slot, NB - 1 + c - w, rows, ls]
                    l = e if l is None else l + e
                    o = ev if o is None else o + ev
                out.append(o * (1.0 / l))
                if len(out) == 2:
                    put_act(ob, c, h, *out)
                yield

    def local_group(g, slot):
        for hh in range(4):
            yield from local_head(slot, hh, 4 * g + hh)

    def prep_task(g):
        nxt = jnp.minimum(g + 1, NG - 1)
        for m in range(7, -1, -1):
            yield from w_prep(m * NG + (nxt if m < 3 else g))

    def layer_a(p):
        def a_body(g, _):
            @pl.when(p == 0)
            def _():
                w_copies(g, lambda cp: cp.wait())

                @pl.when(g + 1 < NG)
                def _():
                    w_copies(g + 1, lambda cp: cp.start())
            _interleave((21 * NB, qkv_a(g)),
                        (128, local_group(jnp.maximum(g - 1, 0), (g + 1) % 2)),
                        (32, prep_task(g)))
            return 0
        lax.fori_loop(0, NG, a_body, 0)

        def a_tail(hh, _):
            _run(local_head((NG - 1) % 2, hh, 4 * (NG - 1) + hh))
            return 0
        lax.fori_loop(0, 4, a_tail, 0)

    def full_step(h, hn):
        for qi in range(NB // 2):
            if hn is not None:
                q = jnp.concatenate([qb[2 * qi + i, _ds(hn, 16), :] for i in range(2)], axis=1)
                z = jnp.zeros_like(q)
                qp = _bf(jnp.concatenate(
                    [jnp.where(hn % 4 == i, q, z) for i in range(4)], axis=0))
            if h is not None:
                mb = mbuf[qi]
            m = l = acc = None
            for j in range(S // 128):
                if h is not None:
                    pieces = [None] * 8
                    for r in reversed(range(8)):
                        e0, e1 = (jnp.exp2(sbuf[qi, _ds(16 * j + 2 * r + i, 8), :] - mb)
                                  for i in range(2))
                        l = e0 + e1 if l is None else l + (e0 + e1)
                        pieces[r] = _pack2(e0, e1)
                    pt = _bf(jnp.concatenate(pieces, axis=0))
                if hn is not None:
                    s = jnp.dot(_bf(kb[hn // 4, _ds(j, 64), :]), qp, preferred_element_type=f32)
                    for r in range(16):
                        sr = s[r * 8:r * 8 + 8]
                        sbuf[qi, _ds(16 * j + r, 8), :] = sr
                        m = sr if m is None else jnp.maximum(m, sr)
                if h is not None:
                    o = jnp.dot(_bf(vb[j // 2, _ds(h, 16), HALF[j % 2]]), pt,
                                preferred_element_type=f32)
                    acc = o if acc is None else acc + o
            if h is not None:
                o = acc * (1.0 / jnp.sum(l, axis=0, keepdims=True))
                for i in range(2):
                    put_act(ob, 2 * qi + i, h, o[:, i * BW:i * BW + 128],
                            o[:, i * BW + 128:(i + 1) * BW])
            if hn is not None:
                mbuf[qi] = jnp.broadcast_to(jnp.max(m, axis=0, keepdims=True), (8, 2 * BW))

    def layer_b():
        def b_body(g, _):
            for c in range(NB):
                def emit_q(i, par, y):
                    qb[c, _ds(2 * g + i, 32), HALF[par]] = _zip16(y * QSCALE)

                def emit_v(i, par, y):
                    vb[c, _ds(2 * g + i, 32), HALF[par]] = pltpu.bitcast(y.astype(bf16), u32)

                held = {}

                def emit_k(i, par, y):
                    held[i, par] = _zip16(y)
                    if i == 0:
                        k = _bf(jnp.concatenate([held[0, par], held[1, par]], axis=0)).T
                        even, odd = _unpack2(pltpu.bitcast(k, u32))
                        k = jnp.stack([even.reshape(8, 8, 128), odd.reshape(8, 8, 128)], axis=1)
                        kb[g, _ds(2 * c + par, 64), :] = pltpu.bitcast(
                            k.reshape(128, 128).astype(bf16), u32)

                _run(proj(BQ + g, xn, c, emit_q))
                _run(proj(BK + g, xn, c, emit_k))
                _run(proj(BV + g, xn, c, emit_v))
            return 0
        lax.fori_loop(0, NG, b_body, 0)

        full_step(None, 0)

        def head_body(h, _):
            full_step(h, h + 1)
            return 0
        lax.fori_loop(0, H - 1, head_body, 0)
        full_step(H - 1, None)

    def period(p, _):
        layernorm_from(jnp.where(p == 0, 0, NB - 1))
        layer_a(p)
        out_proj(AO)
        _run(layernorm(NB - 1))
        layer_b()

        @pl.when(p == 0)
        def _():
            out_proj(BO)
        return 0
    lax.fori_loop(0, 2, period, 0)

    def last_body(f, _):
        for c in range(NB):
            _run(residual(BO + f, c, f))
            u = _pack2(xt[c, _ds(f, 128), HALF[0]], xt[c, _ds(f, 128), HALF[1]])
            xio_u[f, pl.ds(c, 128, stride=NB), :] = u.T
        o_copy(f).start()
        return 0
    lax.fori_loop(0, NG, last_body, 0)
    for f in range(NG):
        o_copy(f).wait()


@jax.jit
def pallas_interleave_layers__sliding_local_dilated__softmax_full_mha__prompt_kernel(
    A_x: jax.Array,
    A_wqkv: jax.Array,
    A_wo: jax.Array,
    B_x: jax.Array,
    B_wqkv: jax.Array,
    B_wo: jax.Array,
):
    del B_x
    sums = pltpu.VMEM((NB, 7, D // 4, 128), u32)
    act = pltpu.VMEM((NB, D // 2, BW), u32)
    out = pl.pallas_call(
        _kernel,
        out_shape=jax.ShapeDtypeStruct((S, D), bf16),
        in_specs=[pl.BlockSpec(memory_space=pl.ANY)] * 5,
        out_specs=pl.BlockSpec(memory_space=pl.ANY),
        scratch_shapes=[
            pltpu.VMEM((NG, S, 128), bf16),
            pltpu.VMEM((8 * NG, D, 128), bf16),
            pltpu.VMEM((8 * NG, 7, 32, D // 2), u32),
            pltpu.VMEM((NB, D, BW), f32),
            sums,
            pltpu.VMEM((2, NB, 128, BW), f32),
            pltpu.VMEM((2, 2 * NB - 1, 128, BW), f32),
            pltpu.VMEM((2, 2 * NB - 1, 128, BW), f32),
            act,
            pltpu.VMEM((NG, S // 2, 128), u32),
            act,
            sums,
            pltpu.VMEM((NB // 2, S, 2 * BW), f32),
            pltpu.VMEM((NB // 2, 8, 2 * BW), f32),
            pltpu.SemaphoreType.DMA((NG,)),
            pltpu.SemaphoreType.DMA((8 * NG,)),
        ],
        compiler_params=pltpu.CompilerParams(vmem_limit_bytes=120 * 2**20),
        name="interleave_layers",
    )(A_x.reshape(S, D), A_wqkv, A_wo, B_wqkv, B_wo)
    return out.reshape(A_x.shape)
```

```python
import math

import jax
import jax.numpy as jnp
from jax import lax
import jax.experimental.pallas as pl
import jax.experimental.pallas.tpu as pltpu

S = 2048
D = 1024
H = 32
DH = D // H
WIN = 8
NB = 8
BW = S // NB
NG = D // 128
EPS = 1e-5
LOG2E = math.log2(math.e)
QSCALE = DH ** -0.5 * LOG2E
NEG = -1e9 * LOG2E

AQ, AK, AV, AO, BQ, BK, BV, BO = (NG * i for i in range(8))

f32, bf16, u32 = jnp.float32, jnp.bfloat16, jnp.uint32
HALF = (slice(0, 128), slice(128, 256))


def _pack2(lo, hi):
    return pltpu.bitcast(pltpu.pack_elementwise([lo, hi], packed_dtype=bf16), u32)


def _unpack2(u):
    return pltpu.bitcast(u << 16, f32), pltpu.bitcast(u & jnp.uint32(0xFFFF0000), f32)


def _zip16(x):
    m, n = x.shape
    x = x.reshape(m // 16, 2, 8, n)
    return _pack2(x[:, 0], x[:, 1]).reshape(m // 2, n)


def _bf(u):
    return pltpu.bitcast(u, bf16)


class _Pacer:
    def __init__(self, loop_index=None):
        self.token = None
        self.never = None if loop_index is None else loop_index * loop_index == 2

    def tie(self, x):
        if self.never is None or self.token is None:
            return x
        tok = self.token if x.dtype == f32 else pltpu.bitcast(self.token, x.dtype)
        tok = jnp.tile(tok, (x.shape[0] // 8, x.shape[1] // 128))
        return jnp.where(self.never, tok, x)

    def run(self, *tasks):
        state = [[0, n, gen] for n, gen in tasks]
        while state:
            t = min(state, key=lambda t: (t[0] + 0.5) / t[1])
            try:
                tok = next(t[2])
            except StopIteration:
                state.remove(t)
                continue
            t[0] += 1
            if tok is not None:
                self.token = tok


_FREE = _Pacer()


def _run(gen):
    for _ in gen:
        pass


def _ds(i, n):
    if isinstance(i, int):
        return pl.ds(i * n, n)
    return pl.ds(pl.multiple_of(i * n, n), n)


def _kernel(x_hbm, awqkv, awo, bwqkv, bwo, o_hbm,
            xio, wraw, wa, wb, wo, xt, xn, qa, ka, va, qb, kb, vb, ob, sbuf, mbuf,
            xsem, wsem):
    w_hbm = (awqkv, awqkv, awqkv, awo, bwqkv, bwqkv, bwqkv, bwo)
    w_off = (0, NG, 2 * NG, 0, 0, NG, 2 * NG, 0)

    def x_copy(f):
        return pltpu.make_async_copy(x_hbm.at[:, _ds(f, 128)], xio.at[f], xsem.at[f])

    def o_copy(f):
        return pltpu.make_async_copy(xio.at[f], o_hbm.at[:, _ds(f, 128)], xsem.at[f])

    def w_copy(m, g):
        return pltpu.make_async_copy(w_hbm[m].at[:, _ds(w_off[m] + g, 128)],
                                     wraw.at[m * NG + g], wsem.at[m * NG + g])

    def w_copies(g, action):
        for m in range(3, 8):
            action(w_copy(m, g))

        @pl.when(g + 1 < NG)
        def _():
            for m in range(3):
                action(w_copy(m, g + 1))

    def w_prep(n, dst, pace=_FREE):
        for t in range(4):
            w = _bf(pace.tie(pltpu.bitcast(wraw[n, 256 * t:256 * t + 256, :], u32)))
            w = w.astype(f32).reshape(8, 4, 8, 128)
            k1, k2 = (pltpu.bitcast(
                _bf(_pack2(w[:, i], w[:, i + 1]).reshape(64, 128)).T, u32) for i in (0, 2))
            ls = slice(128 * t, 128 * t + 128)
            dst[2, :, ls] = k1[:32]
            dst[3, :, ls] = k2[32:]
            a11, a21, a12, a22 = (_unpack2(k) for k in (k1[:32], k1[32:], k2[:32], k2[32:]))
            for r, a, b, op in ((0, a11, a22, jnp.add), (1, a21, a22, jnp.add),
                                (4, a11, a12, jnp.add), (5, a21, a11, jnp.subtract),
                                (6, a12, a22, jnp.subtract)):
                dst[r, :, ls] = _pack2(op(a[0], b[0]), op(a[1], b[1]))
            yield

    def put_act(dst, c, h, even, odd):
        b11, b21, b12, b22 = even[:16], even[16:], odd[:16], odd[16:]
        for r, t in enumerate((b11 + b22, b11, b12 - b22, b21 - b11, b22, b11 + b12, b21 + b22)):
            dst[c, r, _ds(h, 8), :] = _pack2(t[:8], t[8:])

    def proj(w, src, c, emit):
        def mm(r):
            return jnp.dot(_bf(w[r]), _bf(src[c, r]), preferred_element_type=f32)
        m2 = mm(1)
        yield m2[:8]
        m4 = mm(3)
        emit(1, 0, m2 + m4)
        yield m4[:8]
        t22 = mm(5) - m2
        yield t22[:8]
        t11 = mm(6) + m4
        yield t11[:8]
        m1 = mm(0)
        t11, t22 = t11 + m1, t22 + m1
        yield t11[:8]
        m3 = mm(2)
        emit(1, 1, t22 + m3)
        yield m3[:8]
        m5 = mm(4)
        emit(0, 1, m3 + m5)
        emit(0, 0, t11 - m5)
        yield m5[:8]

    for f in range(NG):
        x_copy(f).start()
    for m in range(3):
        w_copy(m, 0).start()

    def zero_body(i, _):
        z = jnp.zeros((128, BW), f32)
        qa[1, jnp.minimum(i, NB - 1)] = z
        ka[1, i] = z
        va[1, i] = z
        return 0
    lax.fori_loop(0, 2 * NB - 1, zero_body, 0)

    xio_u = xio.bitcast(u32)

    def in_body(f, _):
        x_copy(f).wait()
        for c in range(NB):
            even, odd = _unpack2(xio_u[f, pl.ds(c, 128, stride=NB), :].T)
            xt[c, _ds(f, 128), HALF[0]] = even
            xt[c, _ds(f, 128), HALF[1]] = odd
        return 0
    lax.fori_loop(0, NG, in_body, 0)
    w_copies(0, lambda cp: cp.start())
    for m in range(3):
        w_copy(m, 0).wait()
    _FREE.run(*((4, w_prep(m * NG, wa.at[0, m])) for m in range(3)))

    def layernorm(c, pace=_FREE):
        def load(h):
            return xt[c, _ds(h, DH), :].reshape(4, 8, BW)
        acc = None
        for h in range(H):
            x = load(h)
            x = (x[0] + x[1]) + (x[2] + x[3])
            acc = x if acc is None else acc + x
            if h % 4 == 3:
                yield
        mean = jnp.broadcast_to(jnp.sum(acc, axis=0, keepdims=True) * (1.0 / D), (8, BW))
        acc = None
        for h in range(H):
            if h % 2 == 0:
                mean = pace.tie(mean)
            d = load(h) - mean
            d = d * d
            d = (d[0] + d[1]) + (d[2] + d[3])
            acc = d if acc is None else acc + d
            if h % 2 == 1:
                yield
        rstd = lax.rsqrt(jnp.sum(acc, axis=0, keepdims=True) * (1.0 / D) + EPS)
        for h in range(H):
            mean = pace.tie(mean)
            y = (load(h) - mean).reshape(DH, BW) * rstd
            put_act(xn, c, h, y[:, HALF[0]], y[:, HALF[1]])
            yield

    def layernorm_from(first):
        def ln_body(c, _):
            _run(layernorm(c))
            return 0
        lax.fori_loop(first, NB, ln_body, 0)

    def residual(w, c, f):
        def emit(i, par, y):
            xt[c, _ds(2 * f + i, 64), HALF[par]] += y
        return proj(w, ob, c, emit)

    def out_proj(layer):
        def block(c):
            for f in range(NG):
                yield from residual(wo.at[layer * NG + f], c, f)

        def prep(g, pace):
            for m in range(3):
                yield from w_prep(BQ + m * NG + g, wb.at[3 * g + m], pace)

        def out_body(c, _):
            pace = _Pacer(c)
            tasks = [(7 * NG, block(c)), (58, layernorm(jnp.maximum(c - 1, 0), pace))]
            if layer == 0:
                tasks.append((13, prep(c, pace)))
            pace.run(*tasks)
            return 0
        lax.fori_loop(0, NB, out_body, 0)

    def qkv_a(slot):
        for c in range(NB):
            def emit_q(i, par, y):
                qa[slot, c, _ds(i, 64), HALF[par]] = y * QSCALE
            yield from proj(wa.at[slot, 0], xn, c, emit_q)
            for m, dst in ((1, ka), (2, va)):
                def emit_kv(i, par, y):
                    dst[slot, NB - 1 + c, _ds(i, 64), HALF[par]] = y
                    if c > 0:
                        dst[slot, c - 1, _ds(i, 64), HALF[par]] = pltpu.roll(y, 1, 1)
                yield from proj(wa.at[slot, m], xn, c, emit_kv)

    def local_head(slot, hh, h, pace=_FREE):
        first = lax.broadcasted_iota(jnp.int32, (1, 128), 1) == 0
        rows = _ds(hh, DH)
        for c in range(NB):
            out = []
            for ls in HALF:
                q = pace.tie(qa[slot, c, rows, ls])
                t = []
                for w in range(WIN):
                    tw = jnp.sum(q * ka[slot, NB - 1 + c - w, rows, ls], axis=0, keepdims=True)
                    t.append(jnp.where(first, NEG, tw) if c < w else tw)
                m = t[0]
                for w in range(1, WIN):
                    m = jnp.maximum(m, t[w])
                yield
                m = pace.tie(jnp.broadcast_to(m, (8, 128)))
                l = o = None
                for w in range(WIN):
                    e = jnp.exp2(t[w] - m)
                    ev = e * va[slot, NB - 1 + c - w, rows, ls].reshape(4, 8, 128)
                    l = e if l is None else l + e
                    o = ev if o is None else o + ev
                out.append((o * (1.0 / l)).reshape(DH, 128))
                if len(out) == 2:
                    put_act(ob, c, h, *out)
                yield

    def local_group(g, slot, pace):
        for hh in range(4):
            yield from local_head(slot, hh, 4 * g + hh, pace)

    def prep_a(g, slot, pace):
        for m in range(3):
            yield from w_prep(m * NG + (g + 1) % NG, wa.at[slot, m], pace)
        yield from w_prep(AO + g, wo.at[g], pace)

    def layer_a(p):
        def step(g, slot):
            @pl.when(p == 0)
            def _():
                w_copies(g, lambda cp: cp.wait())

                @pl.when(g + 1 < NG)
                def _():
                    w_copies(g + 1, lambda cp: cp.start())
            pace = _Pacer(g)
            pace.run((21 * NB, qkv_a(slot)),
                     (130, local_group(jnp.maximum(g - 1, 0), 1 - slot, pace)),
                     (17, prep_a(g, 1 - slot, pace)))

        def a_body(i, _):
            step(2 * i, 0)
            step(2 * i + 1, 1)
            return 0
        lax.fori_loop(0, NG // 2, a_body, 0)

        def a_tail(hh, _):
            _run(local_head((NG - 1) % 2, hh, 4 * (NG - 1) + hh))
            return 0
        lax.fori_loop(0, 4, a_tail, 0)

    def full_step(h, hn):
        for qi in range(NB // 2):
            if hn is not None:
                q = jnp.concatenate([qb[2 * qi + i, _ds(hn, 16), :] for i in range(2)], axis=1)
                z = jnp.zeros_like(q)
                qp = _bf(jnp.concatenate(
                    [jnp.where(hn % 4 == i, q, z) for i in range(4)], axis=0))
            if h is not None:
                mb = mbuf[qi]
            m = l = acc = None
            for j in range(S // 128):
                if h is not None:
                    pieces = [None] * 8
                    for r in reversed(range(8)):
                        e0, e1 = (jnp.exp2(sbuf[qi, _ds(16 * j + 2 * r + i, 8), :] - mb)
                                  for i in range(2))
                        l = e0 + e1 if l is None else l + (e0 + e1)
                        pieces[r] = _pack2(e0, e1)
                    pt = _bf(jnp.concatenate(pieces, axis=0))
                if hn is not None:
                    s = jnp.dot(_bf(kb[hn // 4, _ds(j, 64), :]), qp, preferred_element_type=f32)
                    for r in range(16):
                        sr = s[r * 8:r * 8 + 8]
                        sbuf[qi, _ds(16 * j + r, 8), :] = sr
                        m = sr if m is None else jnp.maximum(m, sr)
                if h is not None:
                    o = jnp.dot(_bf(vb[j // 2, _ds(h, 16), HALF[j % 2]]), pt,
                                preferred_element_type=f32)
                    acc = o if acc is None else acc + o
            if h is not None:
                o = acc * (1.0 / jnp.sum(l, axis=0, keepdims=True))
                for i in range(2):
                    put_act(ob, 2 * qi + i, h, o[:, i * BW:i * BW + 128],
                            o[:, i * BW + 128:(i + 1) * BW])
            if hn is not None:
                mbuf[qi] = jnp.broadcast_to(jnp.max(m, axis=0, keepdims=True), (8, 2 * BW))

    def layer_b():
        def qkv_b(g):
            for c in range(NB):
                def emit_q(i, par, y):
                    qb[c, _ds(2 * g + i, 32), HALF[par]] = _zip16(y * QSCALE)

                def emit_v(i, par, y):
                    vb[c, _ds(2 * g + i, 32), HALF[par]] = pltpu.bitcast(y.astype(bf16), u32)

                held = {}

                def emit_k(i, par, y):
                    held[i, par] = _zip16(y)
                    if i == 0:
                        k = _bf(jnp.concatenate([held[0, par], held[1, par]], axis=0)).T
                        even, odd = _unpack2(pltpu.bitcast(k, u32))
                        k = jnp.stack([even.reshape(8, 8, 128), odd.reshape(8, 8, 128)], axis=1)
                        kb[g, _ds(2 * c + par, 64), :] = pltpu.bitcast(
                            k.reshape(128, 128).astype(bf16), u32)

                for m, emit in enumerate((emit_q, emit_k, emit_v)):
                    yield from proj(wb.at[3 * g + m], xn, c, emit)

        def b_body(g, _):
            pace = _Pacer(g)
            pace.run((21 * NB, qkv_b(g)), (5, w_prep(BO + g, wo.at[NG + g], pace)))
            return 0
        lax.fori_loop(0, NG, b_body, 0)

        full_step(None, 0)

        def head_body(h, _):
            full_step(h, h + 1)
            return 0
        lax.fori_loop(0, H - 1, head_body, 0)
        full_step(H - 1, None)

    def period(p, _):
        layernorm_from(jnp.where(p == 0, 0, NB - 1))
        layer_a(p)
        out_proj(0)
        _run(layernorm(NB - 1))
        layer_b()

        @pl.when(p == 0)
        def _():
            out_proj(1)
        return 0
    lax.fori_loop(0, 2, period, 0)

    def last_body(f, _):
        for c in range(NB):
            _run(residual(wo.at[NG + f], c, f))
            u = _pack2(xt[c, _ds(f, 128), HALF[0]], xt[c, _ds(f, 128), HALF[1]])
            xio_u[f, pl.ds(c, 128, stride=NB), :] = u.T
        o_copy(f).start()
        return 0
    lax.fori_loop(0, NG, last_body, 0)
    for f in range(NG):
        o_copy(f).wait()


@jax.jit
def pallas_interleave_layers__sliding_local_dilated__softmax_full_mha__prompt_kernel(
    A_x: jax.Array,
    A_wqkv: jax.Array,
    A_wo: jax.Array,
    B_x: jax.Array,
    B_wqkv: jax.Array,
    B_wo: jax.Array,
):
    del B_x
    sums = pltpu.VMEM((NB, 7, D // 4, 128), u32)
    act = pltpu.VMEM((NB, D // 2, BW), u32)
    out = pl.pallas_call(
        _kernel,
        out_shape=jax.ShapeDtypeStruct((S, D), bf16),
        in_specs=[pl.BlockSpec(memory_space=pl.ANY)] * 5,
        out_specs=pl.BlockSpec(memory_space=pl.ANY),
        scratch_shapes=[
            pltpu.VMEM((NG, S, 128), bf16),
            pltpu.VMEM((8 * NG, D, 128), bf16),
            pltpu.VMEM((2, 3, 7, 32, D // 2), u32),
            pltpu.VMEM((3 * NG, 7, 32, D // 2), u32),
            pltpu.VMEM((2 * NG, 7, 32, D // 2), u32),
            pltpu.VMEM((NB, D, BW), f32),
            sums,
            pltpu.VMEM((2, NB, 128, BW), f32),
            pltpu.VMEM((2, 2 * NB - 1, 128, BW), f32),
            pltpu.VMEM((2, 2 * NB - 1, 128, BW), f32),
            act,
            pltpu.VMEM((NG, S // 2, 128), u32),
            act,
            sums,
            pltpu.VMEM((NB // 2, S, 2 * BW), f32),
            pltpu.VMEM((NB // 2, 8, 2 * BW), f32),
            pltpu.SemaphoreType.DMA((NG,)),
            pltpu.SemaphoreType.DMA((8 * NG,)),
        ],
        compiler_params=pltpu.CompilerParams(vmem_limit_bytes=120 * 2**20),
        name="interleave_layers",
    )(A_x.reshape(S, D), A_wqkv, A_wo, B_wqkv, B_wo)
    return out.reshape(A_x.shape)
```

```python
import math

import jax
import jax.numpy as jnp
from jax import lax
import jax.experimental.pallas as pl
import jax.experimental.pallas.tpu as pltpu

S = 2048
D = 1024
H = 32
DH = D // H
WIN = 8
NB = 8
BW = S // NB
NG = D // 128
EPS = 1e-5
LOG2E = math.log2(math.e)
QSCALE = DH ** -0.5 * LOG2E
NEG = -1e9 * LOG2E

AQ, AK, AV, AO, BQ, BK, BV, BO = (NG * i for i in range(8))

LQ, LK, LV, LN = 0, 2 * NB - 1, 4 * NB - 2, 5 * NB

f32, bf16, u32 = jnp.float32, jnp.bfloat16, jnp.uint32
HALF = (slice(0, 128), slice(128, 256))


def _pack2(lo, hi):
    return pltpu.bitcast(pltpu.pack_elementwise([lo, hi], packed_dtype=bf16), u32)


def _unpack2(u):
    return pltpu.bitcast(u << 16, f32), pltpu.bitcast(u & jnp.uint32(0xFFFF0000), f32)


def _zip16(x):
    m, n = x.shape
    x = x.reshape(m // 16, 2, 8, n)
    return _pack2(x[:, 0], x[:, 1]).reshape(m // 2, n)


def _bf(u):
    return pltpu.bitcast(u, bf16)


class _Pacer:
    def __init__(self, loop_index=None):
        self.token = None
        self.never = None if loop_index is None else loop_index * loop_index == 2

    def tie(self, x):
        if self.never is None or self.token is None:
            return x
        tok = self.token if x.dtype == f32 else pltpu.bitcast(self.token, x.dtype)
        tok = jnp.tile(tok, (x.shape[0] // 8, x.shape[1] // 128))
        return jnp.where(self.never, tok, x)

    def run(self, *tasks):
        state = [[0, n, gen] for n, gen in tasks]
        while state:
            t = min(state, key=lambda t: (t[0] + (1.0 if t is state[0] else 0.0)) / t[1])
            try:
                tok = next(t[2])
            except StopIteration:
                state.remove(t)
                continue
            t[0] += 1
            if tok is not None:
                self.token = tok


_FREE = _Pacer()


def _run(gen):
    for _ in gen:
        pass


def _ds(i, n):
    if isinstance(i, int):
        return pl.ds(i * n, n)
    return pl.ds(pl.multiple_of(i * n, n), n)


def _kernel(x_hbm, awqkv, awo, bwqkv, bwo, o_hbm,
            xio, wraw, wa, wb, wo, xt, xn, la, qb, kb, vb, ob, hold, sbuf, mbuf,
            xsem, wsem):
    w_hbm = (awqkv, awqkv, awqkv, awo, bwqkv, bwqkv, bwqkv, bwo)
    w_off = (0, NG, 2 * NG, 0, 0, NG, 2 * NG, 0)

    def x_copy(f):
        return pltpu.make_async_copy(x_hbm.at[:, _ds(f, 128)], xio.at[f], xsem.at[f])

    def o_copy(f):
        return pltpu.make_async_copy(xio.at[f], o_hbm.at[:, _ds(f, 128)], xsem.at[f])

    def w_copy(m, g):
        return pltpu.make_async_copy(w_hbm[m].at[:, _ds(w_off[m] + g, 128)],
                                     wraw.at[m * NG + g], wsem.at[m * NG + g])

    def w_copies(g, action):
        for m in range(3, 8):
            action(w_copy(m, g))

        @pl.when(g + 1 < NG)
        def _():
            for m in range(3):
                action(w_copy(m, g + 1))

    def w_prep(n, dst, pace=_FREE):
        for t in range(4):
            w = _bf(pace.tie(pltpu.bitcast(wraw[n, 256 * t:256 * t + 256, :], u32)))
            w = w.astype(f32).reshape(8, 4, 8, 128)
            k1, k2 = (pltpu.bitcast(
                _bf(_pack2(w[:, i], w[:, i + 1]).reshape(64, 128)).T, u32) for i in (0, 2))
            ls = slice(128 * t, 128 * t + 128)
            dst[2, :, ls] = k1[:32]
            dst[3, :, ls] = k2[32:]
            a11, a21, a12, a22 = (_unpack2(k) for k in (k1[:32], k1[32:], k2[:32], k2[32:]))
            for r, a, b, op in ((0, a11, a22, jnp.add), (1, a21, a22, jnp.add),
                                (4, a11, a12, jnp.add), (5, a21, a11, jnp.subtract),
                                (6, a12, a22, jnp.subtract)):
                dst[r, :, ls] = _pack2(op(a[0], b[0]), op(a[1], b[1]))
            yield

    def act_sums(even, odd):
        b11, b21, b12, b22 = even[:16], even[16:], odd[:16], odd[16:]
        return [_pack2(t[:8], t[8:]) for t in
                (b11 + b22, b11, b12 - b22, b21 - b11, b22, b11 + b12, b21 + b22)]

    def put_act(dst, c, h, sums):
        for r, t in enumerate(sums):
            dst[c, r, _ds(h, 8), :] = t

    def proj(w, src, c, emit):
        def mm(r):
            return jnp.dot(_bf(w[r]), _bf(src[c, r]), preferred_element_type=f32)
        m2 = mm(1)
        yield m2[:8]
        m4 = mm(3)
        emit(1, 0, m2 + m4)
        yield m4[:8]
        t22 = mm(5) - m2
        yield t22[:8]
        t11 = mm(6) + m4
        yield t11[:8]
        m1 = mm(0)
        t11, t22 = t11 + m1, t22 + m1
        yield t11[:8]
        m3 = mm(2)
        emit(1, 1, t22 + m3)
        yield m3[:8]
        m5 = mm(4)
        emit(0, 1, m3 + m5)
        emit(0, 0, t11 - m5)
        yield m5[:8]

    for f in range(2):
        x_copy(f).start()

    def zero_body(i, _):
        z = jnp.zeros((128, BW), f32)
        xt[0, _ds(i, 128)] = z
        for j in range(LN // NG):
            la[1, i * (LN // NG) + j] = z
        return 0
    lax.fori_loop(0, NG, zero_body, 0)

    xio_u = xio.bitcast(u32)

    def in_body(f, _):
        x_copy(f).wait()

        @pl.when(f + 2 < NG)
        def _():
            x_copy(f + 2).start()

        @pl.when(f + 2 == NG)
        def _():
            for m in range(3):
                w_copy(m, 0).start()
        for c in range(NB):
            even, odd = _unpack2(xio_u[f, pl.ds(c, 128, stride=NB), :].T)
            xt[c + 1, _ds(f, 128), HALF[0]] = even
            xt[c + 1, _ds(f, 128), HALF[1]] = odd
        return 0
    lax.fori_loop(0, NG, in_body, 0)
    w_copies(0, lambda cp: cp.start())
    for m in range(3):
        w_copy(m, 0).wait()
    _FREE.run(*((4, w_prep(m * NG, wa.at[0, m])) for m in range(3)))

    def layernorm(src, c, pace=_FREE):
        def load(h):
            return xt[src, _ds(h, DH), :].reshape(4, 8, BW)
        acc = None
        for h in range(H):
            x = load(h)
            acc = x[:2] if acc is None else acc + x[:2]
            acc = acc + x[2:]
            if h % 4 == 3:
                yield
                acc = jnp.stack([pace.tie(acc[0]), pace.tie(acc[1])])
        mean = jnp.sum(acc[0] + acc[1], axis=0, keepdims=True) * (1.0 / D)
        mean = jnp.broadcast_to(mean, (8, BW))
        acc = None
        for h in range(H):
            if h % 2 == 0:
                mean = pace.tie(mean)
            d = load(h) - mean
            d = d * d
            d = (d[0] + d[1]) + (d[2] + d[3])
            acc = d if acc is None else acc + d
            if h % 2 == 1:
                yield
        rstd = lax.rsqrt(jnp.sum(acc, axis=0, keepdims=True) * (1.0 / D) + EPS)
        for h in range(H):
            mean = pace.tie(mean)
            y = (load(h) - mean).reshape(DH, BW) * rstd
            put_act(xn, c, h, act_sums(y[:, HALF[0]], y[:, HALF[1]]))
            yield

    def layernorm_from(first):
        def ln_body(c, _):
            _run(layernorm(c + 1, c))
            return 0
        lax.fori_loop(first, NB, ln_body, 0)

    def residual(w, c, f):
        def emit(i, par, y):
            xt[c + 1, _ds(2 * f + i, 64), HALF[par]] += y
        return proj(w, ob, c, emit)

    def qkv_a(slot):
        for c in range(NB):
            for m, base in ((1, LK), (2, LV)):
                def emit_kv(i, par, y):
                    la[slot, base + c, _ds(i, 64), HALF[par]] = y
                    if c > 0:
                        la[slot, base + c - NB, _ds(i, 64), HALF[par]] = pltpu.roll(y, 1, 1)
                yield from proj(wa.at[slot, m], xn, c, emit_kv)

            def emit_q(i, par, y):
                la[slot, LQ + c, _ds(i, 64), HALF[par]] = y * QSCALE
            yield from proj(wa.at[slot, 0], xn, c, emit_q)

    def local(slot, hh, c, emit, pace=_FREE):
        lane = lax.broadcasted_iota(jnp.int32, (1, 128), 1)
        rows = _ds(hh, DH)
        src = la.at[slot, pl.ds(c, LV + 1)]
        out = []
        for ls in HALF:
            q = pace.tie(src[LQ, rows, ls])
            t = []
            for w in range(WIN):
                tw = jnp.sum(q * src[LK - w, rows, ls], axis=0, keepdims=True)
                if w > 0 and (not isinstance(c, int) or c < w):
                    tw = jnp.where(NB * lane + c < w, NEG, tw)
                t.append(tw)
            m = t[0]
            for w in range(1, WIN):
                m = jnp.maximum(m, t[w])
            yield
            m = pace.tie(jnp.broadcast_to(m, (8, 128)))
            l = o = None
            for w in range(WIN):
                e = jnp.exp2(t[w] - m)
                ev = e * src[LV - w, rows, ls].reshape(4, 8, 128)
                l = e if l is None else l + e
                o = ev if o is None else o + ev
            out.append((o * (1.0 / l)).reshape(DH, 128))
            if len(out) == 2:
                emit(act_sums(*out))
            yield

    def local_group(g, slot, blocks, pace=_FREE):
        for hh in range(4):
            for c in blocks:
                yield from local(slot, hh, c, lambda t: put_act(ob, c, 4 * g + hh, t), pace)

    def prep_a(g, slot, pace):
        for m in range(3):
            yield from w_prep(m * NG + (g + 1) % NG, wa.at[slot, m], pace)
        yield from w_prep(AO + g, wo.at[g], pace)

    def layer_a(p):
        def step(g, slot):
            @pl.when(p == 0)
            def _():
                w_copies(g, lambda cp: cp.wait())

                @pl.when(g + 1 < NG)
                def _():
                    w_copies(g + 1, lambda cp: cp.start())
            pace = _Pacer(g)
            pace.run((21 * NB, qkv_a(slot)),
                     (132, local_group(jnp.maximum(g - 1, 0), 1 - slot, range(NB), pace)),
                     (18, prep_a(g, 1 - slot, pace)))

        def a_body(i, _):
            step(2 * i, 0)
            step(2 * i + 1, 1)
            return 0
        lax.fori_loop(0, NG // 2, a_body, 0)
        _run(local_group(NG - 1, 1, [0]))

    def full_step(h, hn, acc=None):
        for qi in range(NB // 2):
            if hn is not None:
                q = jnp.concatenate([qb[2 * qi + i, _ds(hn, 16), :] for i in range(2)], axis=1)
                z = jnp.zeros_like(q)
                qp = _bf(jnp.concatenate(
                    [jnp.where(hn & 3 == i, q, z) for i in range(4)], axis=0))
            if h is not None:
                mb = mbuf[qi]
            m = l = None
            if h is None or hn is None:
                acc = None
            else:
                acc = jnp.where(_Pacer(h).never, acc, 0.0)
            for j in range(S // 128):
                if h is not None:
                    pieces = [None] * 8
                    for r in reversed(range(8)):
                        e0, e1 = (jnp.exp2(sbuf[qi, _ds(16 * j + 2 * r + i, 8), :] - mb)
                                  for i in range(2))
                        l = e0 + e1 if l is None else l + (e0 + e1)
                        pieces[r] = _pack2(e0, e1)
                    pt = _bf(jnp.concatenate(pieces, axis=0))
                if hn is not None:
                    s = jnp.dot(_bf(kb[hn >> 2, _ds(j, 64), :]), qp, preferred_element_type=f32)
                    for r in range(16):
                        sr = s[r * 8:r * 8 + 8]
                        sbuf[qi, _ds(16 * j + r, 8), :] = sr
                        m = sr if m is None else jnp.maximum(m, sr)
                if h is not None:
                    o = jnp.dot(_bf(vb[j // 2, _ds(h, 16), HALF[j % 2]]), pt,
                                preferred_element_type=f32)
                    acc = o if acc is None else acc + o
            if h is not None:
                o = acc * (1.0 / jnp.sum(l, axis=0, keepdims=True))
                for i in range(2):
                    put_act(ob, 2 * qi + i, h, act_sums(o[:, i * BW:i * BW + 128],
                                                        o[:, i * BW + 128:(i + 1) * BW]))
            if hn is not None:
                mbuf[qi] = jnp.broadcast_to(jnp.max(m, axis=0, keepdims=True), (8, 2 * BW))
        return acc

    def layer_b():
        def qkv_b(g):
            for c in range(NB):
                def emit_q(i, par, y):
                    qb[c, _ds(2 * g + i, 32), HALF[par]] = _zip16(y * QSCALE)

                def emit_v(i, par, y):
                    vb[c, _ds(2 * g + i, 32), HALF[par]] = pltpu.bitcast(y.astype(bf16), u32)

                held = {}

                def emit_k(i, par, y):
                    held[i, par] = _zip16(y)
                    if i == 0:
                        k = _bf(jnp.concatenate([held[0, par], held[1, par]], axis=0)).T
                        even, odd = _unpack2(pltpu.bitcast(k, u32))
                        k = jnp.stack([even.reshape(8, 8, 128), odd.reshape(8, 8, 128)], axis=1)
                        kb[g, _ds(2 * c + par, 64), :] = pltpu.bitcast(
                            k.reshape(128, 128).astype(bf16), u32)

                for m, emit in enumerate((emit_q, emit_k, emit_v)):
                    yield from proj(wb.at[3 * g + m], xn, c, emit)

        def b_body(g, _):
            pace = _Pacer(g)
            pace.run((21 * NB, qkv_b(g)), (5, w_prep(BO + g, wo.at[NG + g], pace)))
            return 0
        lax.fori_loop(0, NG, b_body, 0)

        full_step(None, 0)

        def head_body(h, acc):
            return full_step(h, h + 1, acc)
        lax.fori_loop(0, H - 1, head_body, jnp.zeros((DH, 2 * BW), f32))
        full_step(H - 1, None)

    def out_proj(full):
        def block(c):
            for f in range(NG):
                yield from residual(wo.at[full * NG + f], c, f)

        def prep(g, pace):
            for m in range(3):
                yield from w_prep(BQ + m * NG + g, wb.at[3 * g + m], pace)

        def out_body(c, _):
            pace = _Pacer(c)

            def tail():
                for hh in range(4):
                    yield from local(1, hh, jnp.minimum(c + 1, NB - 1),
                                     lambda t: put_act(hold, 0, hh, t), pace)
            pace.run((7 * NG, block(c)), (58, layernorm(c, jnp.maximum(c - 1, 0), pace)),
                     (13, prep(c, pace)), (17, tail()))

            @pl.when(jnp.logical_and(full == 0, c + 1 < NB))
            def _():
                ob[c + 1, :, _ds(NG - 1, 32), :] = hold[0]
            return 0
        lax.fori_loop(0, NB, out_body, 0)

    def layer(i, _):
        layernorm_from(jnp.where(i == 0, 0, NB - 1))
        pl.when(i % 2 == 0)(lambda: layer_a(i))
        pl.when(i % 2 == 1)(layer_b)
        pl.when(i < 3)(lambda: out_proj(i % 2))
        return 0
    lax.fori_loop(0, 4, layer, 0)

    def put_out(f, c):
        u = _pack2(xt[c + 1, _ds(f, 128), HALF[0]], xt[c + 1, _ds(f, 128), HALF[1]])
        xio_u[f, pl.ds(c, 128, stride=NB), :] = u.T

    def last_body(f, _):
        put_out(jnp.maximum(f - 1, 0), NB - 1)
        for c in range(NB):
            _run(residual(wo.at[NG + f], c, f))
            if c < NB - 1:
                put_out(f, c)

        @pl.when(f > 0)
        def _():
            o_copy(f - 1).start()
        return 0
    lax.fori_loop(0, NG, last_body, 0)
    put_out(NG - 1, NB - 1)
    o_copy(NG - 1).start()
    for f in range(NG):
        o_copy(f).wait()


@jax.jit
def pallas_interleave_layers__sliding_local_dilated__softmax_full_mha__prompt_kernel(
    A_x: jax.Array,
    A_wqkv: jax.Array,
    A_wo: jax.Array,
    B_x: jax.Array,
    B_wqkv: jax.Array,
    B_wo: jax.Array,
):
    del B_x
    act = pltpu.VMEM((NB, D // 2, BW), u32)
    out = pl.pallas_call(
        _kernel,
        out_shape=jax.ShapeDtypeStruct((S, D), bf16),
        in_specs=[pl.BlockSpec(memory_space=pl.ANY)] * 5,
        out_specs=pl.BlockSpec(memory_space=pl.ANY),
        scratch_shapes=[
            pltpu.VMEM((NG, S, 128), bf16),
            pltpu.VMEM((8 * NG, D, 128), bf16),
            pltpu.VMEM((2, 3, 7, 32, D // 2), u32),
            pltpu.VMEM((3 * NG, 7, 32, D // 2), u32),
            pltpu.VMEM((2 * NG, 7, 32, D // 2), u32),
            pltpu.VMEM((1 + NB, D, BW), f32),
            pltpu.VMEM((NB, 7, D // 4, 128), u32),
            pltpu.VMEM((2, LN, 128, BW), f32),
            act,
            pltpu.VMEM((NG, S // 2, 128), u32),
            act,
            pltpu.VMEM((NB, 7, D // 4, 128), u32),
            pltpu.VMEM((1, 7, 32, 128), u32),
            pltpu.VMEM((NB // 2, S, 2 * BW), f32),
            pltpu.VMEM((NB // 2, 8, 2 * BW), f32),
            pltpu.SemaphoreType.DMA((NG,)),
            pltpu.SemaphoreType.DMA((8 * NG,)),
        ],
        compiler_params=pltpu.CompilerParams(vmem_limit_bytes=120 * 2**20),
        name="interleave_layers",
    )(A_x.reshape(S, D), A_wqkv, A_wo, B_wqkv, B_wo)
    return out.reshape(A_x.shape)
```

```python
import functools
import math

import jax
import jax.numpy as jnp
from jax import lax
import jax.experimental.pallas as pl
import jax.experimental.pallas.tpu as pltpu

S = 2048
D = 1024
H = 32
DH = D // H
WIN = 8
NB = 8
BW = S // NB
NG = D // 128
EPS = 1e-5
LOG2E = math.log2(math.e)
QSCALE = DH ** -0.5 * LOG2E
NEG = -1e9 * LOG2E

AQ, AK, AV, AO, BQ, BK, BV, BO = (NG * i for i in range(8))

LQ, LK, LV, LN = 0, 2 * NB - 1, 4 * NB - 2, 5 * NB

PREP, LOCAL, NORM = 4 * 190, 410, 200 + 32 * 57
SLACK, LAG_PREP, LAG_LOCAL, LAG_NORM, LAG_ROLL = 6, 10, 9, 7, 12

f32, bf16, u32 = jnp.float32, jnp.bfloat16, jnp.uint32
HALF = (slice(0, 128), slice(128, 256))


def _pack(x):
    return pltpu.bitcast(x.astype(bf16), u32)


def _bf(u):
    return pltpu.bitcast(u, bf16)


class _Pacer:
    def __init__(self, loop_index=None):
        self.token = None
        self.step = 0
        self.due = []
        self.never = None if loop_index is None else loop_index * loop_index == 2

    def tie(self, x):
        if self.never is None or self.token is None:
            return x
        tok = self.token if x.dtype == f32 else pltpu.bitcast(self.token, x.dtype)
        tok = jnp.tile(tok, (x.shape[0] // 8, x.shape[1] // 128))
        return jnp.where(self.never, tok, x)

    def finish(self, u, lag):
        if self.never is not None:
            t = pltpu.bitcast(u, u32)
            t = functools.reduce(jnp.bitwise_or, jnp.split(t, t.shape[1] // 128, axis=1))
            t = functools.reduce(jnp.bitwise_or, jnp.split(t, t.shape[0] // 8, axis=0))
            self.due.append((self.step + lag, t))
            self.due.sort(key=lambda d: d[0])
        return u

    def gate(self, w):
        if not self.due or self.due[0][0] > self.step:
            return w
        corner = w[:8, :128]
        while self.due and self.due[0][0] <= self.step:
            corner = jnp.where(self.never, self.due.pop(0)[1], corner)
        top = jnp.concatenate([corner, w[:8, 128:]], axis=1)
        return jnp.concatenate([top, w[8:]], axis=0)

    def run(self, steps, matmuls, cost, side):
        done = 0
        for step in range(steps):
            self.step = step
            while done * (steps - SLACK) <= step * cost:
                piece = next(side, None)
                if piece is None:
                    break
                done += piece
            self.token = next(matmuls)
        _run(side)
        _run(matmuls)


def _mix(*tasks):
    state = [[0, n, gen] for n, gen in tasks]
    while state:
        t = min(state, key=lambda t: t[0] / t[1])
        piece = next(t[2], None)
        if piece is None:
            state.remove(t)
        else:
            t[0] += piece
            yield piece


_FREE = _Pacer()


def _run(gen):
    for _ in gen:
        pass


def _ds(i, n):
    if isinstance(i, int):
        return pl.ds(i * n, n)
    return pl.ds(pl.multiple_of(i * n, n), n)


def _kernel(x_hbm, awqkv, awo, bwqkv, bwo, o_hbm,
            xio, pairs, wraw, wa, wb, wo, xt, stat, xn, la, qb, kb, vb, ob, hold, sbuf, mbuf,
            xsem, wsem):
    w_hbm = (awqkv, awqkv, awqkv, awo, bwqkv, bwqkv, bwqkv, bwo)
    w_off = (0, NG, 2 * NG, 0, 0, NG, 2 * NG, 0)

    def x_copy(f):
        return pltpu.make_async_copy(x_hbm.at[:, _ds(f, 128)], xio.at[f], xsem.at[f])

    def o_copy(f):
        return pltpu.make_async_copy(xio.at[f], o_hbm.at[:, _ds(f, 128)], xsem.at[f])

    def w_copy(m, g, batch):
        return pltpu.make_async_copy(w_hbm[m].at[:, _ds(w_off[m] + g, 128)],
                                     wraw.at[m * NG + g], wsem.at[batch])

    def w_copies(g, action):
        for m in range(3, 8):
            action(w_copy(m, g, 1))

        @pl.when(g + 1 < NG)
        def _():
            for m in range(3):
                action(w_copy(m, g + 1, 1))

    def w_prep(n, dst, pace=_FREE):
        for t in range(4):
            w = pace.tie(_pack(wraw[n, _ds(t, 256), :])).reshape(8, 2, 8, 128)
            k1, k2 = (_bf(w[:, i].reshape(64, 128)).T for i in range(2))
            dst[2, :, _ds(t, 128)] = _pack(k1)[:32]
            dst[3, :, _ds(t, 128)] = _pack(k2)[32:]
            k1, k2 = k1.astype(f32), k2.astype(f32)
            a11, a21, a12, a22 = k1[:64], k1[64:], k2[:64], k2[64:]
            a = pace.finish(_pack(jnp.concatenate(
                (a11 + a22, a21 + a22, a11 + a12, a21 - a11, a12 - a22), axis=1)), LAG_PREP)
            for i, r in enumerate((0, 1, 4, 5, 6)):
                dst[r, :, _ds(t, 128)] = a[:, 128 * i:128 * i + 128]
            yield PREP // 4

    def act_sums(even, odd):
        b11, b21, b12, b22 = even[:16], even[16:], odd[:16], odd[16:]
        return _pack(jnp.concatenate(
            (b11 + b22, b11, b12 - b22, b21 - b11, b22, b11 + b12, b21 + b22), axis=1))

    def put_act(dst, c, h, sums):
        dst[c, _ds(h, 8), :] = sums

    def proj(w, src, c, emit, pace=_FREE):
        def mm(r):
            return jnp.dot(_bf(pace.gate(w[r])), _bf(src[c, :, _ds(r, 128)]), preferred_element_type=f32)
        m2 = mm(1)
        yield m2[:8]
        m4 = mm(3)
        emit(1, 0, m2 + m4)
        yield m4[:8]
        t22 = mm(5) - m2
        yield t22[:8]
        t11 = mm(6) + m4
        yield t11[:8]
        m1 = mm(0)
        t11, t22 = t11 + m1, t22 + m1
        yield t11[:8]
        m3 = mm(2)
        emit(1, 1, t22 + m3)
        yield m3[:8]
        m5 = mm(4)
        emit(0, 1, m3 + m5)
        emit(0, 0, t11 - m5)
        yield m5[:8]

    def put_x(c, i, par, x):
        xt[c + 1, _ds(i, 64), HALF[par]] = x
        x = x.reshape(8, 8, 128)
        mean = jnp.sum(x, axis=0) * 0.125
        stat[c + 1, 0, _ds(i, 8), HALF[par]] = mean
        stat[c + 1, 1, _ds(i, 8), HALF[par]] = jnp.sum((x - mean) * (x - mean), axis=0)

    for f in range(2):
        x_copy(f).start()

    def zero_body(i, _):
        z = jnp.zeros((128, BW), f32)
        xt[0, _ds(i, 128)] = z
        for j in range(LN // NG):
            la[1, i * (LN // NG) + j] = z
        return 0
    lax.fori_loop(0, NG, zero_body, 0)
    stat[0] = jnp.zeros(stat.shape[1:], f32)

    def in_body(f, _):
        x_copy(f).wait()

        @pl.when(f + 2 < NG)
        def _():
            x_copy(f + 2).start()

        @pl.when(f + 1 == NG)
        def _():
            for m in range(3):
                w_copy(m, 0, 0).start()
        pairs[...] = _pack(xio[f])
        for c in range(NB):
            u = pairs[pl.ds(c, 128, stride=NB), :].T
            for i in range(2):
                put_x(c, 2 * f + i, 0, pltpu.bitcast(u[64 * i:64 * i + 64] << 16, f32))
                put_x(c, 2 * f + i, 1, pltpu.bitcast((u[64 * i:64 * i + 64] >> 16) << 16, f32))
        return 0
    lax.fori_loop(0, NG, in_body, 0)
    w_copies(0, lambda cp: cp.start())

    def layernorm(src, c, pace=_FREE):
        means = stat[src, 0]
        mean = jnp.sum(means, axis=0, keepdims=True) * (8.0 / D)
        d = means - mean
        var = jnp.sum(stat[src, 1] + 8.0 * (d * d), axis=0, keepdims=True) * (1.0 / D)
        rstd = lax.rsqrt(var + EPS)
        mean = jnp.broadcast_to(mean, (8, BW))
        yield 200
        for h in range(H):
            mean = pace.tie(mean)
            y = (xt[src, _ds(h, DH), :].reshape(4, 8, BW) - mean).reshape(DH, BW) * rstd
            put_act(xn, c, h, pace.finish(act_sums(y[:, HALF[0]], y[:, HALF[1]]), LAG_NORM))
            yield 57

    def layernorm_from(first):
        def ln_body(c, _):
            _run(layernorm(c + 1, c))
            return 0
        lax.fori_loop(first, NB, ln_body, 0)

    def qkv_a(slot, pace):
        for c in range(NB):
            for m, base in ((1, LK), (2, LV)):
                def emit_kv(i, par, y):
                    la[slot, base + c, _ds(i, 64), HALF[par]] = y
                    if c > 0:
                        la[slot, base + c - NB, _ds(i, 64), HALF[par]] = pace.finish(
                            pltpu.roll(y, 1, 1), LAG_ROLL)
                yield from proj(wa.at[slot, m], xn, c, emit_kv, pace)

            def emit_q(i, par, y):
                la[slot, LQ + c, _ds(i, 64), HALF[par]] = y * QSCALE
            yield from proj(wa.at[slot, 0], xn, c, emit_q, pace)

    def local(slot, hh, c, emit, pace=_FREE):
        row = lax.broadcasted_iota(jnp.int32, (WIN, 128), 0)
        lane = lax.broadcasted_iota(jnp.int32, (WIN, 128), 1)
        rows = _ds(hh, DH)
        src = la.at[slot, pl.ds(c, LV + 1)]
        out = []
        for ls in HALF:
            q = pace.tie(src[LQ, rows, ls])
            t = [jnp.sum((q * src[LK - w, rows, ls]).reshape(4, 8, 128), axis=0)
                 for w in range(WIN)]
            for step in (1, 2, 4):
                low = row & step == 0
                t = [jnp.where(low, a, b) + pltpu.roll(jnp.where(low, b, a), WIN - step, 0)
                     for a, b in zip(t[::2], t[1::2])]
            t = jnp.where(NB * lane + c < row, NEG, t[0])
            e = jnp.exp2(t - jnp.max(t, axis=0, keepdims=True))
            e = e / jnp.sum(e, axis=0, keepdims=True)
            yield 115
            e = pace.tie(e)
            out.append(functools.reduce(
                jnp.add, (e[w:w + 1] * src[LV - w, rows, ls] for w in range(WIN))))
            if len(out) == 2:
                emit(pace.finish(act_sums(*out), LAG_LOCAL))
            yield 30 + 40 * len(out)

    def local_group(g, slot, blocks, pace=_FREE):
        for c in blocks:
            for hh in range(4):
                yield from local(slot, hh, c, lambda t: put_act(ob, c, 4 * g + hh, t), pace)

    def prep_a(g, slot, pace):
        for m in range(3):
            yield from w_prep(m * NG + (g + 1) % NG, wa.at[slot, m], pace)
        yield from w_prep(AO + g, wo.at[g], pace)
        for m in range(3):
            yield from w_prep(BQ + m * NG + g, wb.at[3 * g + m], pace)

    def layer_a(p):
        def step(g, slot):
            @pl.when(p == 0)
            def _():
                w_copies(g, lambda cp: cp.wait())

                @pl.when(g + 1 < NG)
                def _():
                    w_copies(g + 1, lambda cp: cp.start())
            pace = _Pacer(g)
            pace.run(21 * NB, qkv_a(slot, pace), 32 * LOCAL + 7 * PREP, _mix(
                (32 * LOCAL, local_group(jnp.maximum(g - 1, 0), 1 - slot, range(NB), pace)),
                (7 * PREP, prep_a(g, 1 - slot, pace))))

        def a_body(i, _):
            step(2 * i, 0)
            step(2 * i + 1, 1)
            return 0
        lax.fori_loop(0, NG // 2, a_body, 0)
        _run(local_group(NG - 1, 1, [0]))

    def full_step(h, hn, acc=None):
        for qi in range(NB // 2):
            if hn is not None:
                q = jnp.concatenate([qb[2 * qi + i, _ds(hn, 16), :] for i in range(2)], axis=1)
                z = jnp.zeros_like(q)
                qp = _bf(jnp.concatenate(
                    [jnp.where(hn & 3 == i, q, z) for i in range(4)], axis=0))
            if h is not None:
                mb = mbuf[qi]
            m = l = None
            if h is None or hn is None:
                acc = None
            else:
                acc = jnp.where(_Pacer(h).never, acc, 0.0)
            for j in range(S // 128):
                if h is not None:
                    e = jnp.exp2(sbuf[qi, _ds(j, 128), :].reshape(16, 8, 2 * BW) - mb)
                    for r in reversed(range(0, 16, 2)):
                        l = e[r] + e[r + 1] if l is None else l + (e[r] + e[r + 1])
                    pt = e.reshape(128, 2 * BW).astype(bf16)
                if hn is not None:
                    s = jnp.dot(_bf(kb[hn >> 2, _ds(j, 64), :]), qp, preferred_element_type=f32)
                    sbuf[qi, _ds(j, 128), :] = s
                    for sr in jnp.split(s, 16):
                        m = sr if m is None else jnp.maximum(m, sr)
                if h is not None:
                    o = jnp.dot(_bf(vb[j // 2, _ds(h, 16), HALF[j % 2]]), pt,
                                preferred_element_type=f32)
                    acc = o if acc is None else acc + o
            if h is not None:
                o = acc * (1.0 / jnp.sum(l, axis=0, keepdims=True))
                for i in range(2):
                    put_act(ob, 2 * qi + i, h, act_sums(o[:, i * BW:i * BW + 128],
                                                        o[:, i * BW + 128:(i + 1) * BW]))
            if hn is not None:
                mbuf[qi] = jnp.broadcast_to(jnp.max(m, axis=0, keepdims=True), (8, 2 * BW))
        return acc

    def layer_b():
        def qkv_b(g):
            for c in range(NB):
                def emit_q(i, par, y):
                    qb[c, _ds(2 * g + i, 32), HALF[par]] = _pack(y * QSCALE)

                def emit_v(i, par, y):
                    vb[c, _ds(2 * g + i, 32), HALF[par]] = _pack(y)

                held = {}

                def emit_k(i, par, y):
                    held[i, par] = y
                    if i == 0:
                        k = jnp.concatenate([held[0, par], held[1, par]], axis=0)
                        kb[g, _ds(2 * c + par, 64), :] = _pack(k.astype(bf16).T)

                for m, emit in enumerate((emit_q, emit_k, emit_v)):
                    yield from proj(wb.at[3 * g + m], xn, c, emit)

        def b_body(g, _):
            pace = _Pacer(g)
            pace.run(21 * NB, qkv_b(g), PREP, w_prep(BO + g, wo.at[NG + g], pace))
            return 0
        lax.fori_loop(0, NG, b_body, 0)

        full_step(None, 0)

        def head_body(h, acc):
            return full_step(h, h + 1, acc)
        lax.fori_loop(0, H - 1, head_body, jnp.zeros((DH, 2 * BW), f32))
        full_step(H - 1, None)

    def out_proj(full):
        def block(c, pace):
            for f in range(NG):
                def emit(i, par, y):
                    put_x(c, 2 * f + i, par, xt[c + 1, _ds(2 * f + i, 64), HALF[par]] + y)
                yield from proj(wo.at[full * NG + f], ob, c, emit, pace)

        def out_body(c, _):
            pace = _Pacer(c)

            def tail():
                for hh in range(4):
                    yield from local(1, hh, jnp.minimum(c + 1, NB - 1),
                                     lambda t: put_act(hold, 0, hh, t), pace)
            pace.run(7 * NG, block(c, pace), NORM + 4 * LOCAL, _mix(
                (NORM, layernorm(c, jnp.maximum(c - 1, 0), pace)),
                (4 * LOCAL, tail())))

            @pl.when(jnp.logical_and(full == 0, c + 1 < NB))
            def _():
                ob[c + 1, _ds(NG - 1, 32), :] = hold[0]
            return 0
        lax.fori_loop(0, NB, out_body, 0)

    def layer(i, _):
        layernorm_from(jnp.where(i == 0, 0, NB - 1))

        @pl.when(i == 0)
        def _():
            for m in range(3):
                w_copy(m, 0, 0).wait()
            for m in range(3):
                _run(w_prep(m * NG, wa.at[0, m]))
        pl.when(i % 2 == 0)(lambda: layer_a(i))
        pl.when(i % 2 == 1)(layer_b)
        pl.when(i < 3)(lambda: out_proj(i % 2))
        return 0
    lax.fori_loop(0, 4, layer, 0)

    def last_block(f, c, row, pace=_FREE):
        def emit(i, par, y):
            xt[row, _ds(2 * f + i, 64), HALF[par]] += y
        return proj(wo.at[NG + f], ob, c, emit, pace)

    def last_body(f, _):
        pace = _Pacer(f)

        def blocks():
            for c in range(NB):
                u = pltpu.bitcast(xt[c + 1, _ds(f, 128), :].astype(bf16).astype(f32), u32)
                pairs[pl.ds(c, 128, stride=NB), :] = pace.finish(
                    ((u[:, HALF[0]] >> 16) | u[:, HALF[1]]).T, LAG_PREP)
                if c + 1 < NB:
                    yield from last_block(f, c + 1, c + 2, pace)
            xio[f] = _bf(pairs[...])
            yield from last_block((f + 1) % NG, 0, (f + 1 < NG).astype(jnp.int32), pace)
        pace.run(7 * NB, blocks(), 0, iter(()))
        o_copy(f).start()
        return 0
    _run(last_block(0, 0, 1))
    lax.fori_loop(0, NG, last_body, 0)
    for f in range(NG):
        o_copy(f).wait()


@jax.jit
def pallas_interleave_layers__sliding_local_dilated__softmax_full_mha__prompt_kernel(
    A_x: jax.Array,
    A_wqkv: jax.Array,
    A_wo: jax.Array,
    B_x: jax.Array,
    B_wqkv: jax.Array,
    B_wo: jax.Array,
):
    del B_x
    act = pltpu.VMEM((NB, D // 2, BW), u32)
    out = pl.pallas_call(
        _kernel,
        out_shape=jax.ShapeDtypeStruct((S, D), bf16),
        in_specs=[pl.BlockSpec(memory_space=pl.ANY)] * 5,
        out_specs=pl.BlockSpec(memory_space=pl.ANY),
        scratch_shapes=[
            pltpu.VMEM((NG, S, 128), bf16),
            pltpu.VMEM((S // 2, 128), u32),
            pltpu.VMEM((8 * NG, D, 128), bf16),
            pltpu.VMEM((2, 3, 7, 32, D // 2), u32),
            pltpu.VMEM((3 * NG, 7, 32, D // 2), u32),
            pltpu.VMEM((2 * NG, 7, 32, D // 2), u32),
            pltpu.VMEM((1 + NB, D, BW), f32),
            pltpu.VMEM((1 + NB, 2, D // 8, BW), f32),
            pltpu.VMEM((NB, D // 4, 7 * 128), u32),
            pltpu.VMEM((2, LN, 128, BW), f32),
            act,
            pltpu.VMEM((NG, S // 2, 128), u32),
            act,
            pltpu.VMEM((NB, D // 4, 7 * 128), u32),
            pltpu.VMEM((1, 32, 7 * 128), u32),
            pltpu.VMEM((NB // 2, S, 2 * BW), f32),
            pltpu.VMEM((NB // 2, 8, 2 * BW), f32),
            pltpu.SemaphoreType.DMA((NG,)),
            pltpu.SemaphoreType.DMA((2,)),
        ],
        compiler_params=pltpu.CompilerParams(vmem_limit_bytes=120 * 2**20),
        name="interleave_layers",
    )(A_x.reshape(S, D), A_wqkv, A_wo, B_wqkv, B_wo)
    return out.reshape(A_x.shape)
```

```python
import functools
import math

import jax
import jax.numpy as jnp
from jax import lax
import jax.experimental.pallas as pl
import jax.experimental.pallas.tpu as pltpu

S = 2048
D = 1024
H = 32
DH = D // H
WIN = 8
NB = 8
BW = S // NB
NG = D // 128
EPS = 1e-5
LOG2E = math.log2(math.e)
QSCALE = DH ** -0.5 * LOG2E
NEG = -1e9 * LOG2E

AQ, AK, AV, AO, BQ, BK, BV, BO = (NG * i for i in range(8))

LQ, LK, LV, LN = 0, 2 * NB - 1, 4 * NB - 2, 5 * NB

PREP, LOCAL, NORM = 4 * 190, 410, 200 + 32 * 57
LAG_PREP, LAG_LOCAL, LAG_NORM, LAG_ROLL = 10, 10, 6, 14

f32, bf16, u32 = jnp.float32, jnp.bfloat16, jnp.uint32
HALF = (slice(0, 128), slice(128, 256))


def _pack(x):
    return pltpu.bitcast(x.astype(bf16), u32)


def _bf(u):
    return pltpu.bitcast(u, bf16)


class _Pacer:
    def __init__(self, loop_index=None):
        self.token = None
        self.step = 0
        self.due = []
        self.never = None if loop_index is None else loop_index * loop_index == 2

    def tie(self, x):
        if self.never is None or self.token is None:
            return x
        tok = self.token if x.dtype == f32 else pltpu.bitcast(self.token, x.dtype)
        tok = jnp.tile(tok, (x.shape[0] // 8, x.shape[1] // 128))
        return jnp.where(self.never, tok, x)

    def finish(self, u, lag):
        if self.never is not None:
            t = pltpu.bitcast(u, u32)
            t = functools.reduce(jnp.bitwise_or, jnp.split(t, t.shape[1] // 128, axis=1))
            t = functools.reduce(jnp.bitwise_or, jnp.split(t, t.shape[0] // 8, axis=0))
            self.due.append((self.step + lag, t))
            self.due.sort(key=lambda d: d[0])
        return u

    def gate(self, w):
        if not self.due or self.due[0][0] > self.step:
            return w
        corner = w[:8, :128]
        while self.due and self.due[0][0] <= self.step:
            corner = jnp.where(self.never, self.due.pop(0)[1], corner)
        top = jnp.concatenate([corner, w[:8, 128:]], axis=1)
        return jnp.concatenate([top, w[8:]], axis=0)

    def run(self, steps, matmuls, cost, side, slack=6):
        done = 0
        for step in range(steps):
            self.step = step
            while done * (steps - slack) <= step * cost:
                piece = next(side, None)
                if piece is None:
                    break
                done += piece
            self.token = next(matmuls)
        _run(side)
        _run(matmuls)


def _mix(*tasks):
    state = [[0, n, gen] for n, gen in tasks]
    while state:
        t = min(state, key=lambda t: t[0] / t[1])
        piece = next(t[2], None)
        if piece is None:
            state.remove(t)
        else:
            t[0] += piece
            yield piece


_FREE = _Pacer()


def _run(gen):
    for _ in gen:
        pass


def _ds(i, n):
    if isinstance(i, int):
        return pl.ds(i * n, n)
    return pl.ds(pl.multiple_of(i * n, n), n)


def _kernel(x_hbm, awqkv, awo, bwqkv, bwo, o_hbm,
            xio, pairs, wraw, wa, wb, wo, xt, stat, xn, la, qb, kb, vb, ob, hold, sbuf, mbuf,
            xsem, wsem):
    w_hbm = (awqkv, awqkv, awqkv, awo, bwqkv, bwqkv, bwqkv, bwo)
    w_off = (0, NG, 2 * NG, 0, 0, NG, 2 * NG, 0)

    def x_copy(f):
        return pltpu.make_async_copy(x_hbm.at[:, _ds(f, 128)], xio.at[f], xsem.at[f])

    def o_copy(f):
        return pltpu.make_async_copy(xio.at[f], o_hbm.at[:, _ds(f, 128)], xsem.at[f])

    def w_copy(m, g, batch):
        return pltpu.make_async_copy(w_hbm[m].at[:, _ds(w_off[m] + g, 128)],
                                     wraw.at[m * NG + g], wsem.at[batch])

    def w_copies(g, action):
        for m in range(3, 8):
            action(w_copy(m, g, 1))

        @pl.when(g + 1 < NG)
        def _():
            for m in range(3):
                action(w_copy(m, g + 1, 1))

    def w_prep(n, dst, pace=_FREE):
        for t in range(4):
            w = pace.tie(_pack(wraw[n, _ds(t, 256), :])).reshape(8, 2, 8, 128)
            k1, k2 = (_bf(w[:, i].reshape(64, 128)).T for i in range(2))
            dst[2, :, _ds(t, 128)] = _pack(k1)[:32]
            dst[3, :, _ds(t, 128)] = _pack(k2)[32:]
            k1, k2 = k1.astype(f32), k2.astype(f32)
            a11, a21, a12, a22 = k1[:64], k1[64:], k2[:64], k2[64:]
            a = pace.finish(_pack(jnp.concatenate(
                (a11 + a22, a21 + a22, a11 + a12, a21 - a11, a12 - a22), axis=1)), LAG_PREP)
            for i, r in enumerate((0, 1, 4, 5, 6)):
                dst[r, :, _ds(t, 128)] = a[:, 128 * i:128 * i + 128]
            yield PREP // 4

    def act_sums(even, odd):
        b11, b21, b12, b22 = even[:16], even[16:], odd[:16], odd[16:]
        return _pack(jnp.concatenate(
            (b11 + b22, b11, b12 - b22, b21 - b11, b22, b11 + b12, b21 + b22), axis=1))

    def put_act(dst, c, h, sums):
        dst[c, _ds(h, 8), :] = sums

    def proj(w, src, c, emit, pace=_FREE):
        def mm(r):
            return jnp.dot(_bf(pace.gate(w[r])), _bf(src[c, :, _ds(r, 128)]), preferred_element_type=f32)
        m2 = mm(1)
        yield m2[:8]
        m4 = mm(3)
        emit(1, 0, m2 + m4)
        yield m4[:8]
        t22 = mm(5) - m2
        yield t22[:8]
        t11 = mm(6) + m4
        yield t11[:8]
        m1 = mm(0)
        t11, t22 = t11 + m1, t22 + m1
        yield t11[:8]
        m3 = mm(2)
        emit(1, 1, t22 + m3)
        yield m3[:8]
        m5 = mm(4)
        emit(0, 1, m3 + m5)
        emit(0, 0, t11 - m5)
        yield m5[:8]

    def put_x(c, i, par, x):
        xt[c + 1, _ds(i, 64), HALF[par]] = x
        x = x.reshape(8, 8, 128)
        mean = jnp.sum(x, axis=0) * 0.125
        stat[c + 1, 0, _ds(i, 8), HALF[par]] = mean
        stat[c + 1, 1, _ds(i, 8), HALF[par]] = jnp.sum((x - mean) * (x - mean), axis=0)

    for f in range(2):
        x_copy(f).start()

    def zero_body(i, _):
        z = jnp.zeros((128, BW), f32)
        xt[0, _ds(i, 128)] = z
        for j in range(LN // NG):
            la[1, i * (LN // NG) + j] = z
        return 0
    lax.fori_loop(0, NG, zero_body, 0)
    stat[0] = jnp.zeros(stat.shape[1:], f32)

    def in_body(f, _):
        x_copy(f).wait()

        @pl.when(f + 2 < NG)
        def _():
            x_copy(f + 2).start()

        @pl.when(f + 1 == NG)
        def _():
            for m in range(3):
                w_copy(m, 0, 0).start()
        pairs[:S // 2] = _pack(xio[f])
        for c in range(NB):
            u = pairs[pl.ds(c, 128, stride=NB), :].T
            for i in range(2):
                put_x(c, 2 * f + i, 0, pltpu.bitcast(u[64 * i:64 * i + 64] << 16, f32))
                put_x(c, 2 * f + i, 1, pltpu.bitcast((u[64 * i:64 * i + 64] >> 16) << 16, f32))
        return 0
    lax.fori_loop(0, NG, in_body, 0)
    w_copies(0, lambda cp: cp.start())

    def layernorm(src, c, pace=_FREE):
        means = stat[src, 0]
        mean = jnp.sum(means, axis=0, keepdims=True) * (8.0 / D)
        d = means - mean
        var = jnp.sum(stat[src, 1] + 8.0 * (d * d), axis=0, keepdims=True) * (1.0 / D)
        rstd = lax.rsqrt(var + EPS)
        mean = jnp.broadcast_to(mean, (8, BW))
        yield 200
        for h in range(H):
            mean = pace.tie(mean)
            y = (xt[src, _ds(h, DH), :].reshape(4, 8, BW) - mean).reshape(DH, BW) * rstd
            put_act(xn, c, h, pace.finish(act_sums(y[:, HALF[0]], y[:, HALF[1]]), LAG_NORM))
            yield 57

    def layernorm_from(first):
        def ln_body(c, _):
            _run(layernorm(c + 1, c))
            return 0
        lax.fori_loop(first, NB, ln_body, 0)

    def qkv_a(slot, pace):
        for c in range(NB):
            for m, base in ((1, LK), (2, LV)):
                def emit_kv(i, par, y):
                    la[slot, base + c, _ds(i, 64), HALF[par]] = y
                    if c > 0:
                        la[slot, base + c - NB, _ds(i, 64), HALF[par]] = pace.finish(
                            pltpu.roll(y, 1, 1), LAG_ROLL)
                yield from proj(wa.at[slot, m], xn, c, emit_kv, pace)

            def emit_q(i, par, y):
                la[slot, LQ + c, _ds(i, 64), HALF[par]] = y * QSCALE
            yield from proj(wa.at[slot, 0], xn, c, emit_q, pace)

    def local(slot, hh, c, emit, pace=_FREE):
        row = lax.broadcasted_iota(jnp.int32, (WIN, 128), 0)
        lane = lax.broadcasted_iota(jnp.int32, (WIN, 128), 1)
        rows = _ds(hh, DH)
        src = la.at[slot, pl.ds(c, LV + 1)]
        out = []
        for ls in HALF:
            q = pace.tie(src[LQ, rows, ls])
            t = [jnp.sum((q * src[LK - w, rows, ls]).reshape(4, 8, 128), axis=0)
                 for w in range(WIN)]
            for step in (1, 2, 4):
                low = row & step == 0
                t = [jnp.where(low, a, b) + pltpu.roll(jnp.where(low, b, a), WIN - step, 0)
                     for a, b in zip(t[::2], t[1::2])]
            t = jnp.where(NB * lane + c < row, NEG, t[0])
            e = jnp.exp2(t - jnp.max(t, axis=0, keepdims=True))
            e = e / jnp.sum(e, axis=0, keepdims=True)
            yield 115
            e = pace.tie(e)
            out.append(functools.reduce(
                jnp.add, (e[w:w + 1] * src[LV - w, rows, ls] for w in range(WIN))))
            if len(out) == 2:
                emit(pace.finish(act_sums(*out), LAG_LOCAL))
            yield 30 + 40 * len(out)

    def local_group(g, slot, blocks, pace=_FREE):
        for hh in range(4):
            for c in blocks:
                yield from local(slot, hh, c, lambda t: put_act(ob, c, 4 * g + hh, t), pace)

    def prep_a(g, slot, pace):
        for m in range(3):
            yield from w_prep(m * NG + (g + 1) % NG, wa.at[slot, m], pace)
        yield from w_prep(AO + g, wo.at[g], pace)
        for m in range(3):
            yield from w_prep(BQ + m * NG + g, wb.at[3 * g + m], pace)

    def layer_a(p):
        def step(g, slot):
            @pl.when(p == 0)
            def _():
                w_copies(g, lambda cp: cp.wait())

                @pl.when(g + 1 < NG)
                def _():
                    w_copies(g + 1, lambda cp: cp.start())
            pace = _Pacer(g)
            pace.run(21 * NB, qkv_a(slot, pace), 32 * LOCAL + 7 * PREP, _mix(
                (32 * LOCAL, local_group(jnp.maximum(g - 1, 0), 1 - slot, range(NB), pace)),
                (7 * PREP, prep_a(g, 1 - slot, pace))), slack=6)

        def a_body(i, _):
            step(2 * i, 0)
            step(2 * i + 1, 1)
            return 0
        lax.fori_loop(0, NG // 2, a_body, 0)
        _run(local_group(NG - 1, 1, [0]))

    def full_step(h, hn, acc=None):
        for qi in range(NB // 2):
            if hn is not None:
                q = jnp.concatenate([qb[2 * qi + i, _ds(hn, 16), :] for i in range(2)], axis=1)
                z = jnp.zeros_like(q)
                qp = _bf(jnp.concatenate(
                    [jnp.where(hn & 3 == i, q, z) for i in range(4)], axis=0))
            if h is not None:
                mb = mbuf[qi]
            m = l = None
            if h is None or hn is None:
                acc = None
            else:
                acc = jnp.where(_Pacer(h).never, acc, 0.0)
            for j in range(S // 128):
                if h is not None:
                    e = jnp.exp2(sbuf[qi, _ds(j, 128), :].reshape(16, 8, 2 * BW) - mb)
                    for r in reversed(range(0, 16, 2)):
                        l = e[r] + e[r + 1] if l is None else l + (e[r] + e[r + 1])
                    pt = e.reshape(128, 2 * BW).astype(bf16)
                if hn is not None:
                    s = jnp.dot(_bf(kb[hn >> 2, _ds(j, 64), :]), qp, preferred_element_type=f32)
                    sbuf[qi, _ds(j, 128), :] = s
                    for sr in jnp.split(s, 16):
                        m = sr if m is None else jnp.maximum(m, sr)
                if h is not None:
                    o = jnp.dot(_bf(vb[j // 2, _ds(h, 16), HALF[j % 2]]), pt,
                                preferred_element_type=f32)
                    acc = o if acc is None else acc + o
            if h is not None:
                o = acc * (1.0 / jnp.sum(l, axis=0, keepdims=True))
                for i in range(2):
                    put_act(ob, 2 * qi + i, h, act_sums(o[:, i * BW:i * BW + 128],
                                                        o[:, i * BW + 128:(i + 1) * BW]))
            if hn is not None:
                mbuf[qi] = jnp.broadcast_to(jnp.max(m, axis=0, keepdims=True), (8, 2 * BW))
        return acc

    def layer_b():
        def qkv_b(g):
            for c in range(NB):
                def emit_q(i, par, y):
                    qb[c, _ds(2 * g + i, 32), HALF[par]] = _pack(y * QSCALE)

                def emit_v(i, par, y):
                    vb[c, _ds(2 * g + i, 32), HALF[par]] = _pack(y)

                held = {}

                def emit_k(i, par, y):
                    held[i, par] = y
                    if i == 0:
                        k = jnp.concatenate([held[0, par], held[1, par]], axis=0)
                        kb[g, _ds(2 * c + par, 64), :] = _pack(k.astype(bf16).T)

                for m, emit in enumerate((emit_q, emit_k, emit_v)):
                    yield from proj(wb.at[3 * g + m], xn, c, emit)

        def b_body(g, _):
            pace = _Pacer(g)
            pace.run(21 * NB, qkv_b(g), PREP, w_prep(BO + g, wo.at[NG + g], pace))
            return 0
        lax.fori_loop(0, NG, b_body, 0)

        full_step(None, 0)

        def head_body(h, acc):
            return full_step(h, h + 1, acc)
        lax.fori_loop(0, H - 1, head_body, jnp.zeros((DH, 2 * BW), f32))
        full_step(H - 1, None)

    def out_proj(full):
        def block(c, pace):
            for f in range(NG):
                def emit(i, par, y):
                    put_x(c, 2 * f + i, par, xt[c + 1, _ds(2 * f + i, 64), HALF[par]] + y)
                yield from proj(wo.at[full * NG + f], ob, c, emit, pace)

        def out_body(c, _):
            pace = _Pacer(c)

            def tail():
                for hh in range(4):
                    yield from local(1, hh, jnp.minimum(c + 1, NB - 1),
                                     lambda t: put_act(hold, 0, hh, t), pace)
            pace.run(7 * NG, block(c, pace), NORM + 4 * LOCAL, _mix(
                (NORM, layernorm(c, jnp.maximum(c - 1, 0), pace)),
                (4 * LOCAL, tail())), slack=9)

            @pl.when(jnp.logical_and(full == 0, c + 1 < NB))
            def _():
                ob[c + 1, _ds(NG - 1, 32), :] = hold[0]
            return 0
        lax.fori_loop(0, NB, out_body, 0)

    def layer(i, _):
        layernorm_from(jnp.where(i == 0, 0, NB - 1))

        @pl.when(i == 0)
        def _():
            for m in range(3):
                w_copy(m, 0, 0).wait()
            for m in range(3):
                _run(w_prep(m * NG, wa.at[0, m]))
        pl.when(i % 2 == 0)(lambda: layer_a(i))
        pl.when(i % 2 == 1)(layer_b)
        pl.when(i < 3)(lambda: out_proj(i % 2))
        return 0
    lax.fori_loop(0, 4, layer, 0)

    def last_block(f, c, row, pace=_FREE):
        def emit(i, par, y):
            xt[row, _ds(2 * f + i, 64), HALF[par]] += y
        return proj(wo.at[NG + f], ob, c, emit, pace)

    def last_body(f, _):
        pace = _Pacer(f)

        def blocks():
            for c in range(NB):
                u = pltpu.bitcast(xt[c + 1, _ds(f, 128), :].astype(bf16).astype(f32), u32)
                pairs[pl.ds(c, 128, stride=NB), :] = pace.finish(
                    ((u[:, HALF[0]] >> 16) | u[:, HALF[1]]).T, LAG_PREP)
                if c + 2 < NB:
                    yield from last_block(f, c + 2, c + 3, pace)
            for c in range(2):
                for i, tok in enumerate(last_block(
                        (f + 1) % NG, c, jnp.where(f + 1 < NG, c + 1, 0), pace), 7 * c - 2):
                    yield tok
                    if 0 <= i < 8:
                        xio[f, _ds(i, S // 8)] = _bf(pace.tie(pairs[_ds(i, S // 16)]))
        pace.run(7 * NB, blocks(), 0, iter(()))
        o_copy(f).start()
        return 0
    for c in range(2):
        _run(last_block(0, c, c + 1))
    lax.fori_loop(0, NG, last_body, 0)
    for f in range(NG):
        o_copy(f).wait()


@jax.jit
def pallas_interleave_layers__sliding_local_dilated__softmax_full_mha__prompt_kernel(
    A_x: jax.Array,
    A_wqkv: jax.Array,
    A_wo: jax.Array,
    B_x: jax.Array,
    B_wqkv: jax.Array,
    B_wo: jax.Array,
):
    del B_x
    act = pltpu.VMEM((NB, D // 2, BW), u32)
    out = pl.pallas_call(
        _kernel,
        out_shape=jax.ShapeDtypeStruct((S, D), bf16),
        in_specs=[pl.BlockSpec(memory_space=pl.ANY)] * 5,
        out_specs=pl.BlockSpec(memory_space=pl.ANY),
        scratch_shapes=[
            pltpu.VMEM((NG, S, 128), bf16),
            pltpu.VMEM((S // 2 + NB, 128), u32),
            pltpu.VMEM((8 * NG, D, 128), bf16),
            pltpu.VMEM((2, 3, 7, 32, D // 2), u32),
            pltpu.VMEM((3 * NG, 7, 32, D // 2), u32),
            pltpu.VMEM((2 * NG, 7, 32, D // 2), u32),
            pltpu.VMEM((1 + NB, D, BW), f32),
            pltpu.VMEM((1 + NB, 2, D // 8, BW), f32),
            pltpu.VMEM((NB, D // 4, 7 * 128), u32),
            pltpu.VMEM((2, LN, 128, BW), f32),
            act,
            pltpu.VMEM((NG, S // 2, 128), u32),
            act,
            pltpu.VMEM((NB, D // 4, 7 * 128), u32),
            pltpu.VMEM((1, 32, 7 * 128), u32),
            pltpu.VMEM((NB // 2, S, 2 * BW), f32),
            pltpu.VMEM((NB // 2, 8, 2 * BW), f32),
            pltpu.SemaphoreType.DMA((NG,)),
            pltpu.SemaphoreType.DMA((2,)),
        ],
        compiler_params=pltpu.CompilerParams(vmem_limit_bytes=120 * 2**20),
        name="interleave_layers",
    )(A_x.reshape(S, D), A_wqkv, A_wo, B_wqkv, B_wo)
    return out.reshape(A_x.shape)
```

```python
import functools
import math

import jax
import jax.numpy as jnp
from jax import lax
import jax.experimental.pallas as pl
import jax.experimental.pallas.tpu as pltpu

S = 2048
D = 1024
H = 32
DH = D // H
WIN = 8
NB = 8
BW = S // NB
NG = D // 128
EPS = 1e-5
LOG2E = math.log2(math.e)
QSCALE = DH ** -0.5 * LOG2E
NEG = -1e9 * LOG2E

AQ, AK, AV, AO, BQ, BK, BV, BO = (NG * i for i in range(8))

LQ, LK, LV, LN = 0, 2 * NB - 1, 4 * NB - 2, 5 * NB

PREP, LOCAL, NORM = 4 * 190, 410, 200 + 32 * 57
LAG_PREP, LAG_LOCAL, LAG_NORM, LAG_ROLL = 10, 10, 6, 14

f32, bf16, u32 = jnp.float32, jnp.bfloat16, jnp.uint32
HALF = (slice(0, 128), slice(128, 256))


def _pack(x):
    return pltpu.bitcast(x.astype(bf16), u32)


def _bf(u):
    return pltpu.bitcast(u, bf16)


def _halves(x, n):
    rows, cols = x.shape
    x = x.reshape(rows // (2 * n), 2, n, cols)
    return x[:, 0].reshape(rows // 2, cols), x[:, 1].reshape(rows // 2, cols)


class _Pacer:
    def __init__(self, loop_index=None):
        self.token = None
        self.step = 0
        self.due = []
        self.never = None if loop_index is None else loop_index * loop_index == 2

    def tie(self, x):
        if self.never is None or self.token is None:
            return x
        tok = self.token if x.dtype == f32 else pltpu.bitcast(self.token, x.dtype)
        tok = jnp.tile(tok, (x.shape[0] // 8, x.shape[1] // 128))
        return jnp.where(self.never, tok, x)

    def finish(self, u, lag):
        if self.never is not None:
            t = pltpu.bitcast(u, u32)
            t = functools.reduce(jnp.bitwise_or, jnp.split(t, t.shape[1] // 128, axis=1))
            t = functools.reduce(jnp.bitwise_or, jnp.split(t, t.shape[0] // 8, axis=0))
            self.due.append((self.step + lag, t))
            self.due.sort(key=lambda d: d[0])
        return u

    def gate(self, w):
        if not self.due or self.due[0][0] > self.step:
            return w
        corner = w[:8, :128]
        while self.due and self.due[0][0] <= self.step:
            corner = jnp.where(self.never, self.due.pop(0)[1], corner)
        top = jnp.concatenate([corner, w[:8, 128:]], axis=1)
        return jnp.concatenate([top, w[8:]], axis=0)

    def run(self, steps, matmuls, cost, side, slack=6):
        done = 0
        for step in range(steps):
            self.step = step
            while done * (steps - slack) <= step * cost:
                piece = next(side, None)
                if piece is None:
                    break
                done += piece
            self.token = next(matmuls)
        _run(side)
        _run(matmuls)


def _mix(*tasks):
    state = [[0, n, gen] for n, gen in tasks]
    while state:
        t = min(state, key=lambda t: t[0] / t[1])
        piece = next(t[2], None)
        if piece is None:
            state.remove(t)
        else:
            t[0] += piece
            yield piece


_FREE = _Pacer()


def _run(gen):
    for _ in gen:
        pass


def _ds(i, n):
    if isinstance(i, int):
        return pl.ds(i * n, n)
    return pl.ds(pl.multiple_of(i * n, n), n)


def _kernel(x_hbm, awqkv, awo, bwqkv, bwo, o_hbm,
            xio, pairs, wraw, wa, wb, wo, xt, stat, xn, la, qb, kb, vb, ob, hold, sbuf, mbuf,
            xsem, wsem):
    w_hbm = (awqkv, awqkv, awqkv, awo, bwqkv, bwqkv, bwqkv, bwo)
    w_off = (0, NG, 2 * NG, 0, 0, NG, 2 * NG, 0)

    def x_copy(f):
        return pltpu.make_async_copy(x_hbm.at[:, _ds(f, 128)], xio.at[f], xsem.at[f])

    def o_copy(f):
        return pltpu.make_async_copy(xio.at[f], o_hbm.at[:, _ds(f, 128)], xsem.at[f])

    def w_copy(m, g, batch):
        return pltpu.make_async_copy(w_hbm[m].at[:, _ds(w_off[m] + g, 128)],
                                     wraw.at[m * NG + g], wsem.at[batch])

    def w_copies(g, action):
        for m in range(3, 8):
            action(w_copy(m, g, 1))

        @pl.when(g + 1 < NG)
        def _():
            for m in range(3):
                action(w_copy(m, g + 1, 1))

    def w_prep(n, dst, pace=_FREE):
        for t in range(4):
            w = pace.tie(_pack(wraw[n, _ds(t, 256), :]))
            k1, k2 = (_bf(k).T for k in _halves(w, 8))
            dst[2, :, _ds(t, 128)] = _halves(_pack(k1), 8)[0]
            dst[3, :, _ds(t, 128)] = _halves(_pack(k2), 8)[1]
            (a11, a21), (a12, a22) = (_halves(k.astype(f32), 16) for k in (k1, k2))
            a = pace.finish(_pack(jnp.concatenate(
                (a11 + a22, a21 + a22, a11 + a12, a21 - a11, a12 - a22), axis=1)), LAG_PREP)
            for i, r in enumerate((0, 1, 4, 5, 6)):
                dst[r, :, _ds(t, 128)] = a[:, 128 * i:128 * i + 128]
            yield PREP // 4

    def act_sums(even, odd):
        b11, b21, b12, b22 = even[:16], even[16:], odd[:16], odd[16:]
        return _pack(jnp.concatenate(
            (b11 + b22, b11, b12 - b22, b21 - b11, b22, b11 + b12, b21 + b22), axis=1))

    def put_act(dst, c, h, sums):
        dst[c, _ds(h, 8), :] = sums

    def proj(w, src, c, emit, pace=_FREE):
        def mm(r):
            return jnp.dot(_bf(pace.gate(w[r])), _bf(src[c, :, _ds(r, 128)]),
                           preferred_element_type=f32)
        m2 = mm(1)
        yield m2[:8]
        m4 = mm(3)
        emit(1, 0, m2 + m4)
        yield m4[:8]
        t22 = mm(5) - m2
        yield t22[:8]
        t11 = mm(6) + m4
        yield t11[:8]
        m1 = mm(0)
        t11, t22 = t11 + m1, t22 + m1
        yield t11[:8]
        m3 = mm(2)
        emit(1, 1, t22 + m3)
        yield m3[:8]
        m5 = mm(4)
        emit(0, 1, m3 + m5)
        emit(0, 0, t11 - m5)
        yield m5[:8]

    def put_x(c, f, i, par, x):
        xt[c + 1, i, _ds(f, 64), HALF[par]] = x
        x = x.reshape(8, 8, 128)
        mean = jnp.sum(x, axis=0) * 0.125
        stat[c + 1, 0, _ds(2 * f + i, 8), HALF[par]] = mean
        stat[c + 1, 1, _ds(2 * f + i, 8), HALF[par]] = jnp.sum(jnp.square(x - mean), axis=0)

    for f in range(2):
        x_copy(f).start()

    def zero_body(i, _):
        z = jnp.zeros((2, 64, BW), f32)
        xt[0, :, _ds(i, 64)] = z
        for j in range(LN // NG):
            la[1, i * (LN // NG) + j] = z
        return 0
    lax.fori_loop(0, NG, zero_body, 0)
    stat[0] = jnp.zeros(stat.shape[1:], f32)

    def in_body(f, _):
        x_copy(f).wait()

        @pl.when(f + 2 < NG)
        def _():
            x_copy(f + 2).start()

        @pl.when(f + 1 == NG)
        def _():
            for m in range(3):
                w_copy(m, 0, 0).start()
        pairs[:S // 2] = _pack(xio[f])
        for c in range(NB):
            for i, u in enumerate(_halves(pairs[pl.ds(c, 128, stride=NB), :].T, 16)):
                put_x(c, f, i, 0, pltpu.bitcast(u << 16, f32))
                put_x(c, f, i, 1, pltpu.bitcast((u >> 16) << 16, f32))
        return 0
    lax.fori_loop(0, NG, in_body, 0)
    w_copies(0, lambda cp: cp.start())

    def layernorm(src, c, pace=_FREE):
        means = stat[src, 0]
        mean = jnp.sum(means, axis=0, keepdims=True) * (8.0 / D)
        d = means - mean
        var = jnp.sum(stat[src, 1] + 8.0 * (d * d), axis=0, keepdims=True) * (1.0 / D)
        rstd = lax.rsqrt(var + EPS)
        mean = jnp.broadcast_to(mean, (8, BW))
        yield 200
        for h in range(H):
            mean = pace.tie(mean)
            y = (xt[src, :, _ds(h, 16), :].reshape(4, 8, BW) - mean).reshape(DH, BW) * rstd
            put_act(xn, c, h, pace.finish(act_sums(y[:, HALF[0]], y[:, HALF[1]]), LAG_NORM))
            yield 57

    def layernorm_from(first):
        def ln_body(c, _):
            _run(layernorm(c + 1, c))
            return 0
        lax.fori_loop(first, NB, ln_body, 0)

    def qkv_a(slot, pace):
        for c in range(NB):
            for m, base in ((1, LK), (2, LV)):
                def emit_kv(i, par, y):
                    la[slot, base + c, i, :, HALF[par]] = y
                    if c > 0:
                        la[slot, base + c - NB, i, :, HALF[par]] = pace.finish(
                            pltpu.roll(y, 1, 1), LAG_ROLL)
                yield from proj(wa.at[slot, m], xn, c, emit_kv, pace)

            def emit_q(i, par, y):
                la[slot, LQ + c, i, :, HALF[par]] = y * QSCALE
            yield from proj(wa.at[slot, 0], xn, c, emit_q, pace)

    def local(slot, hh, c, emit, pace=_FREE):
        row = lax.broadcasted_iota(jnp.int32, (WIN, 128), 0)
        lane = lax.broadcasted_iota(jnp.int32, (WIN, 128), 1)
        out = []
        for ls in HALF:
            def load(block):
                return la[slot, c + block, :, _ds(hh, 16), ls].reshape(DH, 128)
            q = pace.tie(load(LQ))
            t = [jnp.sum((q * load(LK - w)).reshape(4, 8, 128), axis=0) for w in range(WIN)]
            for step in (1, 2, 4):
                low = row & step == 0
                t = [jnp.where(low, a, b) + pltpu.roll(jnp.where(low, b, a), WIN - step, 0)
                     for a, b in zip(t[::2], t[1::2])]
            t = jnp.where(NB * lane + c < row, NEG, t[0])
            e = jnp.exp2(t - jnp.max(t, axis=0, keepdims=True))
            e = e / jnp.sum(e, axis=0, keepdims=True)
            yield 115
            e = pace.tie(e)
            out.append(functools.reduce(
                jnp.add, (e[w:w + 1] * load(LV - w) for w in range(WIN))))
            if len(out) == 2:
                emit(pace.finish(act_sums(*out), LAG_LOCAL))
            yield 30 + 40 * len(out)

    def local_group(g, slot, blocks, pace=_FREE):
        for hh in range(4):
            for c in blocks:
                yield from local(slot, hh, c, lambda t: put_act(ob, c, 4 * g + hh, t), pace)

    def prep_a(g, slot, pace):
        for m in range(3):
            yield from w_prep(m * NG + (g + 1) % NG, wa.at[slot, m], pace)
        yield from w_prep(AO + g, wo.at[g], pace)
        for m in range(3):
            yield from w_prep(BQ + m * NG + g, wb.at[3 * g + m], pace)

    def layer_a(p):
        def step(g, slot):
            @pl.when(p == 0)
            def _():
                w_copies(g, lambda cp: cp.wait())

                @pl.when(g + 1 < NG)
                def _():
                    w_copies(g + 1, lambda cp: cp.start())
            pace = _Pacer(g)
            pace.run(21 * NB, qkv_a(slot, pace), 32 * LOCAL + 7 * PREP, _mix(
                (32 * LOCAL, local_group(jnp.maximum(g - 1, 0), 1 - slot, range(NB), pace)),
                (7 * PREP, prep_a(g, 1 - slot, pace))), slack=6)

        def a_body(i, _):
            step(2 * i, 0)
            step(2 * i + 1, 1)
            return 0
        lax.fori_loop(0, NG // 2, a_body, 0)
        _run(local_group(NG - 1, 1, [0]))

    def full_step(h, hn, acc=None):
        for qi in range(NB // 2):
            if hn is not None:
                q = jnp.concatenate([qb[2 * qi + i, hn] for i in range(2)], axis=1)
                qp = _bf(jnp.concatenate([jnp.where(hn & 3 == hh, half, jnp.zeros_like(half))
                                          for half in (q[:8], q[8:]) for hh in range(4)], axis=0))
            if h is not None:
                mb = mbuf[qi]
            m = l = None
            if h is None or hn is None:
                acc = None
            else:
                acc = jnp.where(_Pacer(h).never, acc, 0.0)
            for j in range(S // 128):
                if h is not None:
                    e = jnp.exp2(sbuf[qi, _ds(j, 128), :].reshape(16, 8, 2 * BW) - mb)
                    for r in reversed(range(0, 16, 2)):
                        l = e[r] + e[r + 1] if l is None else (l + e[r + 1]) + e[r]
                    pt = e.reshape(128, 2 * BW).astype(bf16)
                if hn is not None:
                    s = jnp.dot(_bf(kb[hn >> 2, _ds(j, 64), :]), qp, preferred_element_type=f32)
                    sbuf[qi, _ds(j, 128), :] = s
                    s = jnp.max(s.reshape(16, 8, 2 * BW), axis=0)
                    m = s if m is None else jnp.maximum(m, s)
                if h is not None:
                    o = jnp.dot(_bf(vb[j // 2, h, :, HALF[j % 2]]), pt,
                                preferred_element_type=f32)
                    acc = o if acc is None else acc + o
            if h is not None:
                o = acc * (1.0 / jnp.sum(l, axis=0, keepdims=True))
                for i in range(2):
                    put_act(ob, 2 * qi + i, h, act_sums(o[:, i * BW:i * BW + 128],
                                                        o[:, i * BW + 128:(i + 1) * BW]))
            if hn is not None:
                mbuf[qi] = jnp.broadcast_to(jnp.max(m, axis=0, keepdims=True), (8, 2 * BW))
        return acc

    def layer_b():
        def qkv_b(g):
            for c in range(NB):
                def emit_q(i, par, y):
                    qb[c, _ds(g, 4), _ds(i, 8), HALF[par]] = _pack(y * QSCALE).reshape(4, 8, 128)

                def emit_v(i, par, y):
                    vb[c, _ds(g, 4), _ds(i, 8), HALF[par]] = _pack(y).reshape(4, 8, 128)

                held = {}

                def emit_k(i, par, y):
                    held[i, par] = y
                    if i == 0:
                        k = jnp.concatenate([held[0, par], held[1, par]], axis=0)
                        kb[g, _ds(2 * c + par, 64), :] = _pack(k.astype(bf16).T)

                for m, emit in enumerate((emit_q, emit_k, emit_v)):
                    yield from proj(wb.at[3 * g + m], xn, c, emit)

        def b_body(g, _):
            pace = _Pacer(g)
            pace.run(21 * NB, qkv_b(g), PREP, w_prep(BO + g, wo.at[NG + g], pace))
            return 0
        lax.fori_loop(0, NG, b_body, 0)

        full_step(None, 0)

        def head_body(h, acc):
            return full_step(h, h + 1, acc)
        lax.fori_loop(0, H - 1, head_body, jnp.zeros((DH, 2 * BW), f32))
        full_step(H - 1, None)

    def out_proj(full):
        def block(c, pace):
            for f in range(NG):
                def emit(i, par, y):
                    put_x(c, f, i, par, xt[c + 1, i, _ds(f, 64), HALF[par]] + y)
                yield from proj(wo.at[full * NG + f], ob, c, emit, pace)

        def out_body(c, _):
            pace = _Pacer(c)

            def tail():
                for hh in range(4):
                    yield from local(1, hh, jnp.minimum(c + 1, NB - 1),
                                     lambda t: put_act(hold, 0, hh, t), pace)
            pace.run(7 * NG, block(c, pace), NORM + 4 * LOCAL, _mix(
                (NORM, layernorm(c, jnp.maximum(c - 1, 0), pace)),
                (4 * LOCAL, tail())), slack=9)

            @pl.when(jnp.logical_and(full == 0, c + 1 < NB))
            def _():
                ob[c + 1, _ds(NG - 1, 32), :] = hold[0]
            return 0
        lax.fori_loop(0, NB, out_body, 0)

    def layer(i, _):
        layernorm_from(jnp.where(i == 0, 0, NB - 1))

        @pl.when(i == 0)
        def _():
            for m in range(3):
                w_copy(m, 0, 0).wait()
            for m in range(3):
                _run(w_prep(m * NG, wa.at[0, m]))
        pl.when(i % 2 == 0)(lambda: layer_a(i))
        pl.when(i % 2 == 1)(layer_b)
        pl.when(i < 3)(lambda: out_proj(i % 2))
        return 0
    lax.fori_loop(0, 4, layer, 0)

    def last_block(f, c, row, pace=_FREE):
        def emit(i, par, y):
            xt[row, i, _ds(f, 64), HALF[par]] += y
        return proj(wo.at[NG + f], ob, c, emit, pace)

    def last_body(f, _):
        pace = _Pacer(f)

        def blocks():
            for c in range(NB):
                x = jnp.stack([xt[c + 1, i, _ds(f, 64), :].reshape(4, 16, BW) for i in range(2)],
                              axis=1).reshape(128, BW)
                u = pltpu.bitcast(x.astype(bf16).astype(f32), u32)
                pairs[pl.ds(c, 128, stride=NB), :] = pace.finish(
                    ((u[:, HALF[0]] >> 16) | u[:, HALF[1]]).T, LAG_PREP)
                if c + 2 < NB:
                    yield from last_block(f, c + 2, c + 3, pace)
            for c in range(2):
                for i, tok in enumerate(last_block(
                        (f + 1) % NG, c, jnp.where(f + 1 < NG, c + 1, 0), pace), 7 * c - 2):
                    yield tok
                    if 0 <= i < 8:
                        xio[f, _ds(i, S // 8)] = _bf(pace.tie(pairs[_ds(i, S // 16)]))
        pace.run(7 * NB, blocks(), 0, iter(()))
        o_copy(f).start()
        return 0
    for c in range(2):
        _run(last_block(0, c, c + 1))
    lax.fori_loop(0, NG, last_body, 0)
    for f in range(NG):
        o_copy(f).wait()


@jax.jit
def pallas_interleave_layers__sliding_local_dilated__softmax_full_mha__prompt_kernel(
    A_x: jax.Array,
    A_wqkv: jax.Array,
    A_wo: jax.Array,
    B_x: jax.Array,
    B_wqkv: jax.Array,
    B_wo: jax.Array,
):
    del B_x
    act = pltpu.VMEM((NB, H, 16, BW), u32)
    out = pl.pallas_call(
        _kernel,
        out_shape=jax.ShapeDtypeStruct((S, D), bf16),
        in_specs=[pl.BlockSpec(memory_space=pl.ANY)] * 5,
        out_specs=pl.BlockSpec(memory_space=pl.ANY),
        scratch_shapes=[
            pltpu.VMEM((NG, S, 128), bf16),
            pltpu.VMEM((S // 2 + 32, 128), u32),
            pltpu.VMEM((8 * NG, D, 128), bf16),
            pltpu.VMEM((2, 3, 7, 32, D // 2), u32),
            pltpu.VMEM((3 * NG, 7, 32, D // 2), u32),
            pltpu.VMEM((2 * NG, 7, 32, D // 2), u32),
            pltpu.VMEM((1 + NB, 2, D // 2, BW), f32),
            pltpu.VMEM((1 + NB, 2, D // 8, BW), f32),
            pltpu.VMEM((NB, D // 4, 7 * 128), u32),
            pltpu.VMEM((2, LN, 2, 64, BW), f32),
            act,
            pltpu.VMEM((NG, S // 2, 128), u32),
            act,
            pltpu.VMEM((NB, D // 4, 7 * 128), u32),
            pltpu.VMEM((1, 32, 7 * 128), u32),
            pltpu.VMEM((NB // 2, S, 2 * BW), f32),
            pltpu.VMEM((NB // 2, 8, 2 * BW), f32),
            pltpu.SemaphoreType.DMA((NG,)),
            pltpu.SemaphoreType.DMA((2,)),
        ],
        compiler_params=pltpu.CompilerParams(vmem_limit_bytes=120 * 2**20),
        name="interleave_layers",
    )(A_x.reshape(S, D), A_wqkv, A_wo, B_wqkv, B_wo)
    return out.reshape(A_x.shape)
```

```python
import functools
import math

import jax
import jax.numpy as jnp
from jax import lax
import jax.experimental.pallas as pl
import jax.experimental.pallas.tpu as pltpu

S = 2048
D = 1024
H = 32
DH = D // H
WIN = 8
NB = 8
BW = S // NB
NG = D // 128
EPS = 1e-5
LOG2E = math.log2(math.e)
QSCALE = DH ** -0.5 * LOG2E
NEG = -1e9 * LOG2E

AQ, AK, AV, AO, BQ, BK, BV, BO = (NG * i for i in range(8))

LQ, LK, LV, LN = 0, 2 * NB - 1, 4 * NB - 2, 5 * NB

PREP, LOCAL, NORM = 4 * 190, 410, 200 + 32 * 57
LAG_PREP, LAG_LOCAL, LAG_NORM, LAG_ROLL = 10, 10, 6, 14

f32, bf16, u32 = jnp.float32, jnp.bfloat16, jnp.uint32
HALF = (slice(0, 128), slice(128, 256))


def _pack(x):
    return pltpu.bitcast(x.astype(bf16), u32)


def _bf(u):
    return pltpu.bitcast(u, bf16)


def _halves(x, n):
    rows, cols = x.shape
    x = x.reshape(rows // (2 * n), 2, n, cols)
    return x[:, 0].reshape(rows // 2, cols), x[:, 1].reshape(rows // 2, cols)


class _Pacer:
    def __init__(self, loop_index=None):
        self.token = None
        self.step = 0
        self.due = []
        self.never = None if loop_index is None else loop_index * loop_index == 2

    def tie(self, x):
        if self.never is None or self.token is None:
            return x
        tok = self.token if x.dtype == f32 else pltpu.bitcast(self.token, x.dtype)
        tok = jnp.tile(tok, (x.shape[0] // 8, x.shape[1] // 128))
        return jnp.where(self.never, tok, x)

    def finish(self, u, lag):
        if self.never is not None:
            t = pltpu.bitcast(u, u32)
            t = functools.reduce(jnp.bitwise_or, jnp.split(t, t.shape[1] // 128, axis=1))
            t = functools.reduce(jnp.bitwise_or, jnp.split(t, t.shape[0] // 8, axis=0))
            self.due.append((self.step + lag, t))
            self.due.sort(key=lambda d: d[0])
        return u

    def gate(self, w):
        if not self.due or self.due[0][0] > self.step:
            return w
        corner = w[:8, :128]
        while self.due and self.due[0][0] <= self.step:
            corner = jnp.where(self.never, self.due.pop(0)[1], corner)
        top = jnp.concatenate([corner, w[:8, 128:]], axis=1)
        return jnp.concatenate([top, w[8:]], axis=0)

    def run(self, steps, matmuls, cost, side, slack=6):
        done = 0
        for step in range(steps):
            self.step = step
            while done * (steps - slack) <= step * cost:
                piece = next(side, None)
                if piece is None:
                    break
                done += piece
            self.token = next(matmuls)
        _run(side)
        _run(matmuls)


def _mix(*tasks):
    state = [[0, n, gen] for n, gen in tasks]
    while state:
        t = min(state, key=lambda t: t[0] / t[1])
        piece = next(t[2], None)
        if piece is None:
            state.remove(t)
        else:
            t[0] += piece
            yield piece


_FREE = _Pacer()


def _run(gen):
    for _ in gen:
        pass


def _ds(i, n):
    if isinstance(i, int):
        return pl.ds(i * n, n)
    return pl.ds(pl.multiple_of(i * n, n), n)


def _kernel(x_hbm, awqkv, awo, bwqkv, bwo, o_hbm,
            xio, pairs, wraw, wa, wb, wo, xt, stat, xn, la, qb, kb, vb, ob, hold, sbuf, mbuf,
            xsem, wsem):
    w_hbm = (awqkv, awqkv, awqkv, awo, bwqkv, bwqkv, bwqkv, bwo)
    w_off = (0, NG, 2 * NG, 0, 0, NG, 2 * NG, 0)

    def x_copy(f):
        return pltpu.make_async_copy(x_hbm.at[:, _ds(f, 128)], xio.at[f], xsem.at[f])

    def o_copy(f):
        return pltpu.make_async_copy(xio.at[f], o_hbm.at[:, _ds(f, 128)], xsem.at[f])

    def w_copy(m, g, batch):
        return pltpu.make_async_copy(w_hbm[m].at[:, _ds(w_off[m] + g, 128)],
                                     wraw.at[m * NG + g], wsem.at[batch])

    def w_copies(g, action):
        for m in range(3, 8):
            action(w_copy(m, g, 1))

        @pl.when(g + 1 < NG)
        def _():
            for m in range(3):
                action(w_copy(m, g + 1, 1))

    def w_prep(n, dst, pace=_FREE):
        for t in range(4):
            w = pace.tie(_pack(wraw[n, _ds(t, 256), :]))
            k1, k2 = (_bf(k).T for k in _halves(w, 8))
            dst[2, :, _ds(t, 128)] = _halves(_pack(k1), 8)[0]
            dst[3, :, _ds(t, 128)] = _halves(_pack(k2), 8)[1]
            (a11, a21), (a12, a22) = (_halves(k.astype(f32), 16) for k in (k1, k2))
            a = pace.finish(_pack(jnp.concatenate(
                (a11 + a22, a21 + a22, a11 + a12, a21 - a11, a12 - a22), axis=1)), LAG_PREP)
            for i, r in enumerate((0, 1, 4, 5, 6)):
                dst[r, :, _ds(t, 128)] = a[:, 128 * i:128 * i + 128]
            yield PREP // 4

    def act_sums(even, odd):
        b11, b21, b12, b22 = even[:16], even[16:], odd[:16], odd[16:]
        return _pack(jnp.concatenate(
            (b11 + b22, b11, b12 - b22, b21 - b11, b22, b11 + b12, b21 + b22), axis=1))

    def put_act(dst, c, h, sums):
        dst[c, _ds(h, 8), :] = sums

    def proj(w, src, c, emit, pace=_FREE):
        def mm(r):
            return jnp.dot(_bf(pace.gate(w[r])), _bf(src[c, :, _ds(r, 128)]),
                           preferred_element_type=f32)
        m2 = mm(1)
        yield m2[:8]
        m4 = mm(3)
        emit(1, 0, m2 + m4)
        yield m4[:8]
        t22 = mm(5) - m2
        yield t22[:8]
        t11 = mm(6) + m4
        yield t11[:8]
        m1 = mm(0)
        t11, t22 = t11 + m1, t22 + m1
        yield t11[:8]
        m3 = mm(2)
        emit(1, 1, t22 + m3)
        yield m3[:8]
        m5 = mm(4)
        emit(0, 1, m3 + m5)
        emit(0, 0, t11 - m5)
        yield m5[:8]

    def put_x(c, f, i, par, x):
        xt[c + 1, i, _ds(f, 64), HALF[par]] = x
        x = x.reshape(8, 8, 128)
        mean = jnp.sum(x, axis=0) * 0.125
        stat[c + 1, 0, _ds(2 * f + i, 8), HALF[par]] = mean
        stat[c + 1, 1, _ds(2 * f + i, 8), HALF[par]] = jnp.sum(jnp.square(x - mean), axis=0)

    for f in range(2):
        x_copy(f).start()

    def zero_body(i, _):
        z = jnp.zeros((2, 64, BW), f32)
        xt[0, :, _ds(i, 64)] = z
        for j in range(LN // NG):
            la[1, i * (LN // NG) + j] = z
        return 0
    lax.fori_loop(0, NG, zero_body, 0)
    stat[0] = jnp.zeros(stat.shape[1:], f32)

    def in_body(f, _):
        x_copy(f).wait()

        @pl.when(f + 2 < NG)
        def _():
            x_copy(f + 2).start()

        @pl.when(f + 1 == NG)
        def _():
            for m in range(3):
                w_copy(m, 0, 0).start()
        pairs[:S // 2] = _pack(xio[f])
        for c in range(NB):
            for i, u in enumerate(_halves(pairs[pl.ds(c, 128, stride=NB), :].T, 16)):
                put_x(c, f, i, 0, pltpu.bitcast(u << 16, f32))
                put_x(c, f, i, 1, pltpu.bitcast((u >> 16) << 16, f32))
        return 0
    lax.fori_loop(0, NG, in_body, 0)
    w_copies(0, lambda cp: cp.start())

    def layernorm(src, c, pace=_FREE):
        means = stat[src, 0]
        mean = jnp.sum(means, axis=0, keepdims=True) * (8.0 / D)
        d = means - mean
        var = jnp.sum(stat[src, 1] + 8.0 * (d * d), axis=0, keepdims=True) * (1.0 / D)
        rstd = lax.rsqrt(var + EPS)
        mean = jnp.broadcast_to(mean, (8, BW))
        yield 200
        for h in range(H):
            mean = pace.tie(mean)
            y = (xt[src, :, _ds(h, 16), :].reshape(4, 8, BW) - mean).reshape(DH, BW) * rstd
            put_act(xn, c, h, pace.finish(act_sums(y[:, HALF[0]], y[:, HALF[1]]), LAG_NORM))
            yield 57

    def layernorm_from(first):
        def ln_body(c, _):
            _run(layernorm(c + 1, c))
            return 0
        lax.fori_loop(first, NB, ln_body, 0)

    def qkv_a(slot, pace):
        for c in range(NB):
            for m, base in ((1, LK), (2, LV)):
                def emit_kv(i, par, y):
                    la[slot, base + c, i, :, HALF[par]] = y
                    if c > 0:
                        la[slot, base + c - NB, i, :, HALF[par]] = pace.finish(
                            pltpu.roll(y, 1, 1), LAG_ROLL)
                yield from proj(wa.at[slot, m], xn, c, emit_kv, pace)

            def emit_q(i, par, y):
                la[slot, LQ + c, i, :, HALF[par]] = y * QSCALE
            yield from proj(wa.at[slot, 0], xn, c, emit_q, pace)

    def local(slot, hh, c, emit, pace=_FREE):
        row = lax.broadcasted_iota(jnp.int32, (WIN, 128), 0)
        lane = lax.broadcasted_iota(jnp.int32, (WIN, 128), 1)
        out = []
        for ls in HALF:
            def load(block):
                return la[slot, c + block, :, _ds(hh, 16), ls].reshape(DH, 128)
            q = pace.tie(load(LQ))
            t = [jnp.sum((q * load(LK - w)).reshape(4, 8, 128), axis=0) for w in range(WIN)]
            for step in (1, 2, 4):
                low = row & step == 0
                t = [jnp.where(low, a, b) + pltpu.roll(jnp.where(low, b, a), WIN - step, 0)
                     for a, b in zip(t[::2], t[1::2])]
            t = jnp.where(NB * lane + c < row, NEG, t[0])
            e = jnp.exp2(t - jnp.max(t, axis=0, keepdims=True))
            e = e / jnp.sum(e, axis=0, keepdims=True)
            yield 115
            e = pace.tie(e)
            out.append(functools.reduce(
                jnp.add, (e[w:w + 1] * load(LV - w) for w in range(WIN))))
            if len(out) == 2:
                emit(pace.finish(act_sums(*out), LAG_LOCAL))
            yield 30 + 40 * len(out)

    def local_group(g, slot, blocks, pace=_FREE):
        for hh in range(4):
            for c in blocks:
                yield from local(slot, hh, c, lambda t: put_act(ob, c, 4 * g + hh, t), pace)

    def prep_a(g, slot, pace):
        for m in range(3):
            yield from w_prep(m * NG + (g + 1) % NG, wa.at[slot, m], pace)
        yield from w_prep(AO + g, wo.at[g], pace)
        for m in range(3):
            yield from w_prep(BQ + m * NG + g, wb.at[3 * g + m], pace)

    def layer_a(p):
        def step(g, slot):
            @pl.when(p == 0)
            def _():
                w_copies(g, lambda cp: cp.wait())

                @pl.when(g + 1 < NG)
                def _():
                    w_copies(g + 1, lambda cp: cp.start())
            pace = _Pacer(g)
            pace.run(21 * NB, qkv_a(slot, pace), 32 * LOCAL + 7 * PREP, _mix(
                (32 * LOCAL, local_group(jnp.maximum(g - 1, 0), 1 - slot, range(NB), pace)),
                (7 * PREP, prep_a(g, 1 - slot, pace))), slack=6)

        def a_body(i, _):
            step(2 * i, 0)
            step(2 * i + 1, 1)
            return 0
        lax.fori_loop(0, NG // 2, a_body, 0)
        _run(local_group(NG - 1, 1, [0]))

    def full_step(t, tn, acc=None, side=None):
        for hh in range(4):
            if tn is not None:
                q = jnp.concatenate(
                    [qb[2 * (tn >> 3) + i, 4 * (tn & 7) + hh] for i in range(2)], axis=1)
                qp = _bf(jnp.concatenate([half if x == hh else jnp.zeros_like(half)
                                          for half in (q[:8], q[8:]) for x in range(4)], axis=0))
            if t is not None:
                h = 4 * (t & 7) + hh
                mb = mbuf[hh]
            m = l = None
            if t is None or tn is None:
                acc = None
            else:
                acc = jnp.where(_Pacer(t).never, acc, 0.0)
            for j in range(S // 128):
                if t is not None:
                    e = jnp.exp2(sbuf[hh, _ds(j, 128), :].reshape(16, 8, 2 * BW) - mb)
                    for r in reversed(range(0, 16, 2)):
                        l = e[r] + e[r + 1] if l is None else (l + e[r + 1]) + e[r]
                    pt = e.reshape(128, 2 * BW).astype(bf16)
                if tn is not None:
                    s = jnp.dot(_bf(kb[tn & 7, _ds(j, 64), :]), qp, preferred_element_type=f32)
                    sbuf[hh, _ds(j, 128), :] = s
                    s = jnp.max(s.reshape(16, 8, 2 * BW), axis=0)
                    m = s if m is None else jnp.maximum(m, s)
                if side is not None and j % 8 != 0:
                    next(side)
                if t is not None:
                    o = jnp.dot(_bf(vb[j // 2, h, :, HALF[j % 2]]), pt,
                                preferred_element_type=f32)
                    acc = o if acc is None else acc + o
            if t is not None:
                o = acc * (1.0 / jnp.sum(l, axis=0, keepdims=True))
                for i in range(2):
                    put_act(ob, 2 * (t >> 3) + i, h, act_sums(o[:, i * BW:i * BW + 128],
                                                              o[:, i * BW + 128:(i + 1) * BW]))
            if tn is not None:
                mbuf[hh] = jnp.broadcast_to(jnp.max(m, axis=0, keepdims=True), (8, 2 * BW))
        return acc

    def out_block(full, c, pace=_FREE):
        for f in range(NG):
            def emit(i, par, y):
                put_x(c, f, i, par, xt[c + 1, i, _ds(f, 64), HALF[par]] + y)
            yield from proj(wo.at[full * NG + f], ob, c, emit, pace)

    def layer_b():
        def qkv_b(g):
            for c in range(NB):
                def emit_q(i, par, y):
                    qb[c, _ds(g, 4), _ds(i, 8), HALF[par]] = _pack(y * QSCALE).reshape(4, 8, 128)

                def emit_v(i, par, y):
                    vb[c, _ds(g, 4), _ds(i, 8), HALF[par]] = _pack(y).reshape(4, 8, 128)

                held = {}

                def emit_k(i, par, y):
                    held[i, par] = y
                    if i == 0:
                        k = jnp.concatenate([held[0, par], held[1, par]], axis=0)
                        kb[g, _ds(2 * c + par, 64), :] = _pack(k.astype(bf16).T)

                for m, emit in enumerate((emit_q, emit_k, emit_v)):
                    yield from proj(wb.at[3 * g + m], xn, c, emit)

        def b_body(g, _):
            pace = _Pacer(g)
            pace.run(21 * NB, qkv_b(g), PREP, w_prep(BO + g, wo.at[NG + g], pace))
            return 0
        lax.fori_loop(0, NG, b_body, 0)

        full_step(None, 0)

        def head_body(h, acc):
            return full_step(h, h + 1, acc)
        lax.fori_loop(0, H - 1, head_body, jnp.zeros((DH, 2 * BW), f32))
        rest = out_block(1, 0)
        full_step(H - 1, None, side=rest)
        _run(rest)

    def out_proj(full):
        def out_body(c, _):
            pace = _Pacer(c)

            def tail():
                for hh in range(4):
                    yield from local(1, hh, jnp.minimum(c + 1, NB - 1),
                                     lambda t: put_act(hold, 0, hh, t), pace)
            pace.run(7 * NG, out_block(full, c, pace), NORM + 4 * LOCAL, _mix(
                (NORM, layernorm(c, jnp.maximum(c - 1, 0), pace)),
                (4 * LOCAL, tail())), slack=9)

            @pl.when(jnp.logical_and(full == 0, c + 1 < NB))
            def _():
                ob[c + 1, _ds(NG - 1, 32), :] = hold[0]
            return 0
        lax.fori_loop(full, NB, out_body, 0)

    def layer(i, _):
        layernorm_from(jnp.where(i == 0, 0, NB - 1))

        @pl.when(i == 0)
        def _():
            for m in range(3):
                w_copy(m, 0, 0).wait()
            for m in range(3):
                _run(w_prep(m * NG, wa.at[0, m]))
        pl.when(i % 2 == 0)(lambda: layer_a(i))
        pl.when(i % 2 == 1)(layer_b)
        pl.when(i < 3)(lambda: out_proj(i % 2))
        return 0
    lax.fori_loop(0, 4, layer, 0)

    def last_block(f, c, row, pace=_FREE):
        def emit(i, par, y):
            xt[row, i, _ds(f, 64), HALF[par]] += y
        return proj(wo.at[NG + f], ob, c, emit, pace)

    def last_body(f, _):
        pace = _Pacer(f)

        def blocks():
            for c in range(NB):
                x = jnp.stack([xt[c + 1, i, _ds(f, 64), :].reshape(4, 16, BW) for i in range(2)],
                              axis=1).reshape(128, BW)
                u = pltpu.bitcast(x.astype(bf16).astype(f32), u32)
                pairs[pl.ds(c, 128, stride=NB), :] = pace.finish(
                    ((u[:, HALF[0]] >> 16) | u[:, HALF[1]]).T, LAG_PREP)
                if c + 3 < NB:
                    yield from last_block(f, c + 3, c + 4, pace)
            for c in (1, 2):
                for i, tok in enumerate(last_block(
                        (f + 1) % NG, c, jnp.where(f + 1 < NG, c + 1, 0), pace), 7 * c - 9):
                    yield tok
                    if 0 <= i < 8:
                        xio[f, _ds(i, S // 8)] = _bf(pace.tie(pairs[_ds(i, S // 16)]))
        pace.run(7 * (NB - 1), blocks(), 0, iter(()))
        o_copy(f).start()
        return 0
    for c in (1, 2):
        _run(last_block(0, c, c + 1))
    lax.fori_loop(0, NG, last_body, 0)
    for f in range(NG):
        o_copy(f).wait()


@jax.jit
def pallas_interleave_layers__sliding_local_dilated__softmax_full_mha__prompt_kernel(
    A_x: jax.Array,
    A_wqkv: jax.Array,
    A_wo: jax.Array,
    B_x: jax.Array,
    B_wqkv: jax.Array,
    B_wo: jax.Array,
):
    del B_x
    act = pltpu.VMEM((NB, H, 16, BW), u32)
    out = pl.pallas_call(
        _kernel,
        out_shape=jax.ShapeDtypeStruct((S, D), bf16),
        in_specs=[pl.BlockSpec(memory_space=pl.ANY)] * 5,
        out_specs=pl.BlockSpec(memory_space=pl.ANY),
        scratch_shapes=[
            pltpu.VMEM((NG, S, 128), bf16),
            pltpu.VMEM((S // 2 + 32, 128), u32),
            pltpu.VMEM((8 * NG, D, 128), bf16),
            pltpu.VMEM((2, 3, 7, 32, D // 2), u32),
            pltpu.VMEM((3 * NG, 7, 32, D // 2), u32),
            pltpu.VMEM((2 * NG, 7, 32, D // 2), u32),
            pltpu.VMEM((1 + NB, 2, D // 2, BW), f32),
            pltpu.VMEM((1 + NB, 2, D // 8, BW), f32),
            pltpu.VMEM((NB, D // 4, 7 * 128), u32),
            pltpu.VMEM((2, LN, 2, 64, BW), f32),
            act,
            pltpu.VMEM((NG, S // 2, 128), u32),
            act,
            pltpu.VMEM((NB, D // 4, 7 * 128), u32),
            pltpu.VMEM((1, 32, 7 * 128), u32),
            pltpu.VMEM((NB // 2, S, 2 * BW), f32),
            pltpu.VMEM((NB // 2, 8, 2 * BW), f32),
            pltpu.SemaphoreType.DMA((NG,)),
            pltpu.SemaphoreType.DMA((2,)),
        ],
        compiler_params=pltpu.CompilerParams(vmem_limit_bytes=120 * 2**20),
        name="interleave_layers",
    )(A_x.reshape(S, D), A_wqkv, A_wo, B_wqkv, B_wo)
    return out.reshape(A_x.shape)
```

```python
import functools
import math

import jax
import jax.numpy as jnp
from jax import lax
import jax.experimental.pallas as pl
import jax.experimental.pallas.tpu as pltpu

S = 2048
D = 1024
H = 32
DH = D // H
WIN = 8
NB = 8
BW = S // NB
NG = D // 128
EPS = 1e-5
LOG2E = math.log2(math.e)
QSCALE = DH ** -0.5 * LOG2E
NEG = -1e9 * LOG2E

AQ, AK, AV, AO, BQ, BK, BV, BO = (NG * i for i in range(8))

LQ, LK, LV, LN = 0, 2 * NB - 1, 4 * NB - 2, 5 * NB

PREP, LOCAL, NORM = 4 * 160, 410, 200 + 32 * 57
LAG_PREP, LAG_LOCAL, LAG_NORM, LAG_ROLL = 11, 11, 6, 13

f32, bf16, u32 = jnp.float32, jnp.bfloat16, jnp.uint32
HALF = (slice(0, 128), slice(128, 256))


def _pack(x):
    return pltpu.bitcast(x.astype(bf16), u32)


def _bf(u):
    return pltpu.bitcast(u, bf16)


def _halves(x, n):
    rows, cols = x.shape
    x = x.reshape(rows // (2 * n), 2, n, cols)
    return x[:, 0].reshape(rows // 2, cols), x[:, 1].reshape(rows // 2, cols)


class _Pacer:
    def __init__(self, loop_index=None):
        self.token = None
        self.step = 0
        self.due = []
        self.never = None if loop_index is None else loop_index * loop_index == 2

    def tie(self, x):
        if self.never is None or self.token is None:
            return x
        tok = self.token if x.dtype == f32 else pltpu.bitcast(self.token, x.dtype)
        tok = jnp.tile(tok, (x.shape[0] // 8, x.shape[1] // 128))
        return jnp.where(self.never, tok, x)

    def finish(self, u, lag):
        if self.never is not None:
            t = pltpu.bitcast(u, u32)
            t = functools.reduce(jnp.bitwise_or, jnp.split(t, t.shape[1] // 128, axis=1))
            t = functools.reduce(jnp.bitwise_or, jnp.split(t, t.shape[0] // 8, axis=0))
            self.due.append((self.step + lag, t))
            self.due.sort(key=lambda d: d[0])
        return u

    def gate(self, w):
        if not self.due or self.due[0][0] > self.step:
            return w
        corner = w[:8, :128]
        while self.due and self.due[0][0] <= self.step:
            corner = jnp.where(self.never, self.due.pop(0)[1], corner)
        top = jnp.concatenate([corner, w[:8, 128:]], axis=1)
        return jnp.concatenate([top, w[8:]], axis=0)

    def run(self, steps, matmuls, cost=0, side=iter(()), slack=6):
        done = 0
        for step in range(steps):
            self.step = step
            while done * (steps - slack) <= step * cost:
                piece = next(side, None)
                if piece is None:
                    break
                done += piece
            self.token = next(matmuls)
        _run(side)
        _run(matmuls)


def _mix(*tasks):
    state = [[0, n, gen] for n, gen in tasks]
    while state:
        t = min(state, key=lambda t: t[0] / t[1])
        piece = next(t[2], None)
        if piece is None:
            state.remove(t)
        else:
            t[0] += piece
            yield piece


_FREE = _Pacer()


def _run(gen):
    for _ in gen:
        pass


def _ds(i, n):
    if isinstance(i, int):
        return pl.ds(i * n, n)
    return pl.ds(pl.multiple_of(i * n, n), n)


def _kernel(x_hbm, awqkv, awo, bwqkv, bwo, o_hbm,
            xio, pairs, wraw, wa, wb, wo, xt, stat, xn, la, qb, kb, vb, ob, hold, sbuf, mbuf,
            xsem, wsem):
    w_hbm = (awqkv, awqkv, awqkv, awo, bwqkv, bwqkv, bwqkv, bwo)
    w_off = (0, NG, 2 * NG, 0, 0, NG, 2 * NG, 0)

    def x_copy(f):
        return pltpu.make_async_copy(x_hbm.at[:, _ds(f, 128)], xio.at[f], xsem.at[f])

    def o_copy(f):
        return pltpu.make_async_copy(xio.at[f], o_hbm.at[:, _ds(f, 128)], xsem.at[f])

    def w_copy(m, g, batch):
        return pltpu.make_async_copy(w_hbm[m].at[:, _ds(w_off[m] + g, 128)],
                                     wraw.at[m * NG + g], wsem.at[batch])

    def w_copies(g, action):
        for m in range(3, 8):
            action(w_copy(m, g, 1))

        @pl.when(g + 1 < NG)
        def _():
            for m in range(3):
                action(w_copy(m, g + 1, 1))

    def w_prep(n, dst, pace=_FREE):
        for t in range(4):
            w = pace.tie(_pack(wraw[n, _ds(t, 256), :]))
            k1, k2 = (_bf(k).T for k in _halves(w, 8))
            dst[2, :, _ds(t, 128)] = _halves(_pack(k1), 8)[0]
            dst[3, :, _ds(t, 128)] = _halves(_pack(k2), 8)[1]
            (a11, a21), (a12, a22) = (_halves(k.astype(f32), 16) for k in (k1, k2))
            a = pace.finish(_pack(jnp.concatenate(
                (a11 + a22, a21 + a22, a11 + a12, a21 - a11, a12 - a22), axis=1)), LAG_PREP)
            for i, r in enumerate((0, 1, 4, 5, 6)):
                dst[r, :, _ds(t, 128)] = a[:, 128 * i:128 * i + 128]
            yield PREP // 4

    def act_sums(even, odd):
        b11, b21, b12, b22 = even[:16], even[16:], odd[:16], odd[16:]
        return _pack(jnp.concatenate(
            (b11 + b22, b11, b12 - b22, b21 - b11, b22, b11 + b12, b21 + b22), axis=1))

    def put_act(dst, c, h, sums):
        dst[c, _ds(h, 8), :] = sums

    def proj(w, src, c, emit, pace=_FREE):
        def mm(r):
            return jnp.dot(_bf(pace.gate(w[r])), _bf(src[c, :, _ds(r, 128)]),
                           preferred_element_type=f32)
        m2 = mm(1)
        yield m2[:8]
        m4 = mm(3)
        emit(1, 0, m2 + m4)
        yield m4[:8]
        t22 = mm(5) - m2
        yield t22[:8]
        t11 = mm(6) + m4
        yield t11[:8]
        m1 = mm(0)
        t11, t22 = t11 + m1, t22 + m1
        yield t11[:8]
        m3 = mm(2)
        emit(1, 1, t22 + m3)
        yield m3[:8]
        m5 = mm(4)
        emit(0, 1, m3 + m5)
        emit(0, 0, t11 - m5)
        yield m5[:8]

    def put_x(c, f, i, par, x):
        xt[c + 1, i, _ds(f, 64), HALF[par]] = x
        x = x.reshape(8, 8, 128)
        mean = jnp.sum(x, axis=0) * 0.125
        stat[c + 1, 0, _ds(2 * f + i, 8), HALF[par]] = mean
        stat[c + 1, 1, _ds(2 * f + i, 8), HALF[par]] = jnp.sum(jnp.square(x - mean), axis=0)

    for f in range(2):
        x_copy(f).start()

    def zero_body(i, _):
        z = jnp.zeros((2, 64, BW), f32)
        xt[0, :, _ds(i, 64)] = z
        for j in range(LN // NG):
            la[1, i * (LN // NG) + j] = z
        return 0
    lax.fori_loop(0, NG, zero_body, 0)
    stat[0] = jnp.zeros(stat.shape[1:], f32)

    def in_body(f, _):
        x_copy(f).wait()

        @pl.when(f + 2 < NG)
        def _():
            x_copy(f + 2).start()

        @pl.when(f + 2 == NG)
        def _():
            for m in range(3):
                w_copy(m, 0, 0).start()
        pairs[:S // 2] = _pack(xio[f])
        for c in range(NB):
            for i, u in enumerate(_halves(pairs[pl.ds(c, 128, stride=NB), :].T, 16)):
                put_x(c, f, i, 0, pltpu.bitcast(u << 16, f32))
                put_x(c, f, i, 1, pltpu.bitcast((u >> 16) << 16, f32))
        return 0
    lax.fori_loop(0, NG, in_body, 0)
    w_copies(0, lambda cp: cp.start())

    def layernorm(src, c, pace=_FREE):
        means = stat[src, 0]
        mean = jnp.sum(means, axis=0, keepdims=True) * (8.0 / D)
        d = means - mean
        var = jnp.sum(stat[src, 1] + 8.0 * (d * d), axis=0, keepdims=True) * (1.0 / D)
        rstd = lax.rsqrt(var + EPS)
        mean = jnp.broadcast_to(mean, (8, BW))
        yield 200
        for h in range(H):
            mean = pace.tie(mean)
            y = (xt[src, :, _ds(h, 16), :].reshape(4, 8, BW) - mean).reshape(DH, BW) * rstd
            put_act(xn, c, h, pace.finish(act_sums(y[:, HALF[0]], y[:, HALF[1]]), LAG_NORM))
            yield 57

    def layernorm_from(first):
        def ln_body(c, _):
            _run(layernorm(c + 1, c))
            return 0
        lax.fori_loop(first, NB, ln_body, 0)

    def qkv_a(slot, pace):
        for c in range(NB):
            for m, base in ((1, LK), (2, LV)):
                def emit_kv(i, par, y):
                    la[slot, base + c, i, :, HALF[par]] = y
                    if c > 0:
                        la[slot, base + c - NB, i, :, HALF[par]] = pace.finish(
                            pltpu.roll(y, 1, 1), LAG_ROLL)
                yield from proj(wa.at[slot, m], xn, c, emit_kv, pace)

            def emit_q(i, par, y):
                la[slot, LQ + c, i, :, HALF[par]] = y * QSCALE
            yield from proj(wa.at[slot, 0], xn, c, emit_q, pace)

    def local(slot, hh, c, emit, pace=_FREE):
        row = lax.broadcasted_iota(jnp.int32, (WIN, 128), 0)
        lane = lax.broadcasted_iota(jnp.int32, (WIN, 128), 1)
        out = []
        for ls in HALF:
            def load(block):
                return la[slot, c + block, :, _ds(hh, 16), ls].reshape(DH, 128)
            q = pace.tie(load(LQ))
            t = [jnp.sum((q * load(LK - w)).reshape(4, 8, 128), axis=0) for w in range(WIN)]
            for step in (1, 2, 4):
                low = row & step == 0
                t = [jnp.where(low, a, b) + pltpu.roll(jnp.where(low, b, a), WIN - step, 0)
                     for a, b in zip(t[::2], t[1::2])]
            t = jnp.where(NB * lane + c < row, NEG, t[0])
            e = jnp.exp2(t - jnp.max(t, axis=0, keepdims=True))
            e = e / jnp.sum(e, axis=0, keepdims=True)
            yield 115
            e = pace.tie(e)
            out.append(functools.reduce(
                jnp.add, (e[w:w + 1] * load(LV - w) for w in range(WIN))))
            if len(out) == 2:
                emit(pace.finish(act_sums(*out), LAG_LOCAL))
            yield 30 + 40 * len(out)

    def local_group(g, slot, blocks, pace=_FREE):
        for hh in range(4):
            for c in blocks:
                yield from local(slot, hh, c, lambda t: put_act(ob, c, 4 * g + hh, t), pace)

    def prep_a(g, slot, pace):
        for m in range(3):
            yield from w_prep(m * NG + (g + 1) % NG, wa.at[slot, m], pace)
        yield from w_prep(AO + g, wo.at[g], pace)
        for m in range(3):
            yield from w_prep(BQ + m * NG + g, wb.at[3 * g + m], pace)

    def layer_a(i):
        def step(g, slot):
            @pl.when(i == 0)
            def _():
                w_copies(g, lambda cp: cp.wait())

                @pl.when(g + 1 < NG)
                def _():
                    w_copies(g + 1, lambda cp: cp.start())
            pace = _Pacer(g)
            pace.run(21 * NB, qkv_a(slot, pace), 32 * LOCAL + 7 * PREP, _mix(
                (32 * LOCAL, local_group(jnp.maximum(g - 1, 0), 1 - slot, range(NB), pace)),
                (7 * PREP, prep_a(g, 1 - slot, pace))), slack=9)

        def a_body(n, _):
            step(2 * n, 0)
            step(2 * n + 1, 1)
            return 0
        lax.fori_loop(0, NG // 2, a_body, 0)
        _run(local_group(NG - 1, 1, [0]))

    def padded_q(t, hh):
        q = jnp.concatenate([qb[2 * (t >> 3) + i, 4 * (t & 7) + hh] for i in range(2)], axis=1)
        return _bf(jnp.concatenate([half if x == hh else jnp.zeros_like(half)
                                    for half in (q[:8], q[8:]) for x in range(4)], axis=0))

    def full_step(t, tn, acc=None, side=None):
        for hh in range(4):
            h = 4 * (t & 7) + hh
            mb = mbuf[hh]
            m = l = None
            if tn is None:
                acc = None
            else:
                qp = padded_q(tn, hh)
                acc = jnp.where(_Pacer(t).never, acc, 0.0)
            for j in range(S // 128):
                e = jnp.exp2(sbuf[hh, _ds(j, 128), :].reshape(16, 8, 2 * BW) - mb)
                for r in reversed(range(0, 16, 2)):
                    l = e[r] + e[r + 1] if l is None else (l + e[r + 1]) + e[r]
                if tn is not None:
                    s = jnp.dot(_bf(kb[tn & 7, _ds(j, 64), :]), qp, preferred_element_type=f32)
                    sbuf[hh, _ds(j, 128), :] = s
                    s = jnp.max(s.reshape(16, 8, 2 * BW), axis=0)
                    m = s if m is None else jnp.maximum(m, s)
                elif j % 8 != 0:
                    next(side)
                o = jnp.dot(_bf(vb[j // 2, h, :, HALF[j % 2]]),
                            e.reshape(128, 2 * BW).astype(bf16), preferred_element_type=f32)
                acc = o if acc is None else acc + o
            o = acc * (1.0 / jnp.sum(l, axis=0, keepdims=True))
            for i in range(2):
                put_act(ob, 2 * (t >> 3) + i, h, act_sums(o[:, i * BW:i * BW + 128],
                                                          o[:, i * BW + 128:(i + 1) * BW]))
            if tn is not None:
                mbuf[hh] = jnp.broadcast_to(jnp.max(m, axis=0, keepdims=True), (8, 2 * BW))
        return acc

    def out_block(full, c, pace=_FREE):
        for f in range(NG):
            def emit(i, par, y):
                put_x(c, f, i, par, xt[c + 1, i, _ds(f, 64), HALF[par]] + y)
            yield from proj(wo.at[full * NG + f], ob, c, emit, pace)

    def layer_b():
        def qkv_b(g):
            for c in range(NB):
                def emit_q(i, par, y):
                    qb[c, _ds(g, 4), _ds(i, 8), HALF[par]] = _pack(y * QSCALE).reshape(4, 8, 128)

                def emit_v(i, par, y):
                    vb[c, _ds(g, 4), _ds(i, 8), HALF[par]] = _pack(y).reshape(4, 8, 128)

                held = {}

                def emit_k(i, par, y):
                    held[i, par] = y
                    if i == 0:
                        k = jnp.concatenate([held[0, par], held[1, par]], axis=0)
                        kb[g, _ds(2 * c + par, 64), :] = _pack(k.astype(bf16).T)

                for m, emit in enumerate((emit_q, emit_k, emit_v)):
                    yield from proj(wb.at[3 * g + m], xn, c, emit)

        def b_body(g, _):
            pace = _Pacer(g)
            pace.run(21 * NB, qkv_b(g), PREP, w_prep(BO + g, wo.at[NG + g], pace))
            return 0
        lax.fori_loop(0, NG, b_body, 0)

        mbuf[...] = jnp.full(mbuf.shape, -jnp.inf, f32)

        def first_body(n, _):
            for hh in range(4):
                s = jnp.dot(_bf(kb[0, _ds(n, S // 4), :]), padded_q(0, hh),
                            preferred_element_type=f32)
                sbuf[hh, _ds(n, S // 2), :] = s
                mbuf[hh] = jnp.maximum(mbuf[hh], jnp.max(s, axis=0, keepdims=True))
            return 0
        lax.fori_loop(0, 2, first_body, 0)

        def head_body(t, acc):
            return full_step(t, t + 1, acc)
        lax.fori_loop(0, H - 1, head_body, jnp.zeros((DH, 2 * BW), f32))
        rest = out_block(1, 0)
        full_step(H - 1, None, side=rest)
        _run(rest)

    def out_proj(full):
        def out_body(c, _):
            pace = _Pacer(c)

            def tail():
                for hh in range(4):
                    yield from local(1, hh, jnp.minimum(c + 1, NB - 1),
                                     lambda t: put_act(hold, 0, hh, t), pace)
            pace.run(7 * NG, out_block(full, c, pace), NORM + 4 * LOCAL, _mix(
                (NORM, layernorm(c, jnp.maximum(c - 1, 0), pace)),
                (4 * LOCAL, tail())), slack=8)

            @pl.when(jnp.logical_and(full == 0, c + 1 < NB))
            def _():
                ob[c + 1, _ds(NG - 1, 32), :] = hold[0]
            return 0
        lax.fori_loop(full, NB, out_body, 0)

    def layer(i, _):
        layernorm_from(jnp.where(i == 0, 0, NB - 1))

        @pl.when(i == 0)
        def _():
            for m in range(3):
                w_copy(m, 0, 0).wait()
            for m in range(3):
                _run(w_prep(m * NG, wa.at[0, m]))
        pl.when(i % 2 == 0)(lambda: layer_a(i))
        pl.when(i % 2 == 1)(layer_b)
        pl.when(i < 3)(lambda: out_proj(i % 2))
        return 0
    lax.fori_loop(0, 4, layer, 0)

    def last_block(f, c, row, pace=_FREE):
        def emit(i, par, y):
            xt[row, i, _ds(f, 64), HALF[par]] += y
        return proj(wo.at[NG + f], ob, c, emit, pace)

    def last_body(f, _):
        pace = _Pacer(f)

        def blocks():
            for c in range(NB):
                x = jnp.stack([xt[c + 1, i, _ds(f, 64), :].reshape(4, 16, BW) for i in range(2)],
                              axis=1).reshape(128, BW)
                u = pltpu.bitcast(x.astype(bf16).astype(f32), u32)
                pairs[pl.ds(c, 128, stride=NB), :] = pace.finish(
                    ((u[:, HALF[0]] >> 16) | u[:, HALF[1]]).T, LAG_PREP)
                if c + 3 < NB:
                    yield from last_block(f, c + 3, c + 4, pace)
            for c in (1, 2):
                for i, tok in enumerate(last_block(
                        (f + 1) % NG, c, jnp.where(f + 1 < NG, c + 1, 0), pace), 7 * c - 9):
                    yield tok
                    if 0 <= i < 8:
                        xio[f, _ds(i, S // 8)] = _bf(pace.tie(pairs[_ds(i, S // 16)]))
        pace.run(7 * (NB - 1), blocks())
        o_copy(f).start()
        return 0
    for c in (1, 2):
        _run(last_block(0, c, c + 1))
    lax.fori_loop(0, NG, last_body, 0)
    for f in range(NG):
        o_copy(f).wait()


@jax.jit
def pallas_interleave_layers__sliding_local_dilated__softmax_full_mha__prompt_kernel(
    A_x: jax.Array,
    A_wqkv: jax.Array,
    A_wo: jax.Array,
    B_x: jax.Array,
    B_wqkv: jax.Array,
    B_wo: jax.Array,
):
    del B_x
    act = pltpu.VMEM((NB, H, 16, BW), u32)
    out = pl.pallas_call(
        _kernel,
        out_shape=jax.ShapeDtypeStruct((S, D), bf16),
        in_specs=[pl.BlockSpec(memory_space=pl.ANY)] * 5,
        out_specs=pl.BlockSpec(memory_space=pl.ANY),
        scratch_shapes=[
            pltpu.VMEM((NG, S, 128), bf16),
            pltpu.VMEM((S // 2 + 32, 128), u32),
            pltpu.VMEM((8 * NG, D, 128), bf16),
            pltpu.VMEM((2, 3, 7, 32, D // 2), u32),
            pltpu.VMEM((3 * NG, 7, 32, D // 2), u32),
            pltpu.VMEM((2 * NG, 7, 32, D // 2), u32),
            pltpu.VMEM((1 + NB, 2, D // 2, BW), f32),
            pltpu.VMEM((1 + NB, 2, D // 8, BW), f32),
            pltpu.VMEM((NB, D // 4, 7 * 128), u32),
            pltpu.VMEM((2, LN, 2, 64, BW), f32),
            act,
            pltpu.VMEM((NG, S // 2, 128), u32),
            act,
            pltpu.VMEM((NB, D // 4, 7 * 128), u32),
            pltpu.VMEM((1, 32, 7 * 128), u32),
            pltpu.VMEM((4, S, 2 * BW), f32),
            pltpu.VMEM((4, 8, 2 * BW), f32),
            pltpu.SemaphoreType.DMA((NG,)),
            pltpu.SemaphoreType.DMA((2,)),
        ],
        compiler_params=pltpu.CompilerParams(vmem_limit_bytes=120 * 2**20),
        name="interleave_layers",
    )(A_x.reshape(S, D), A_wqkv, A_wo, B_wqkv, B_wo)
    return out.reshape(A_x.shape)
```
